```python
import jax
import jax.numpy as jnp

def _softmax(x, axis=-1):
    return jax.nn.softmax(x, axis=axis)
def _gelu(x):
    return jax.nn.gelu(x, approximate=True)
def _silu(x):
    return jax.nn.silu(x)
def _sigmoid(x):
    return jax.nn.sigmoid(x)
def _layernorm(x, axis=-1, eps=1e-5):
    m = jnp.mean(x, axis=axis, keepdims=True)
    v = jnp.var(x, axis=axis, keepdims=True)
    return (x - m) / jnp.sqrt(v + eps)
def _scatter_add(tgt, idx, src, axis=0):
    return tgt.at[idx].add(src)
def _segment_sum(src, seg, n):
    return jax.ops.segment_sum(src, seg, n)
class _Rng:
    def __init__(self, key):
        self._k = key
    def _next(self):
        self._k, sub = jax.random.split(self._k)
        return sub
    def normal(self, shape):
        return jax.random.normal(self._next(), shape, dtype=jnp.bfloat16)
    def randint(self, lo, hi, shape):
        return jax.random.randint(self._next(), shape, lo, hi, dtype=jnp.int32)
    def uniform(self, shape, lo=0.0, hi=1.0):
        return jax.random.uniform(self._next(), shape, jnp.bfloat16, lo, hi)
    def permutation(self, n):
        return jax.random.permutation(self._next(), n)


kernel_name = 'parallel_sum__sliding_local_dilated__glu_gated_geglu__prompt'

def setup_inputs():
    _rng = _Rng(jax.random.key(int.from_bytes(__import__("os").urandom(4), "little")))
    _w = (lambda a: (lambda t: t.astype(jnp.bfloat16) if jnp.issubdtype(t.dtype, jnp.floating) else t)(jnp.asarray(a)))
    def _A_setup():
        B, S, D = 1, 2048, 1024
        return {
            "x": _w((lambda *s: _rng.normal(s) * 0.05)(B, S, D)),
            "wqkv": _w((lambda *s: _rng.normal(s) * 0.05)(D, 3 * D)),
            "wo": _w((lambda *s: _rng.normal(s) * 0.05)(D, D)),
        }
    _A_in = _A_setup()

    def _B_setup():
        B, S, Dm, Df = 1, 2048, 1024, 3584
        return {
            "x": _w((lambda *s: _rng.normal(s) * 0.05)(B, S, Dm)),
            "w_gate": _w((lambda *s: _rng.normal(s) * 0.05)(Dm, Df) * (Dm ** -0.5)),
            "w_up": _w((lambda *s: _rng.normal(s) * 0.05)(Dm, Df) * (Dm ** -0.5)),
            "w_down": _w((lambda *s: _rng.normal(s) * 0.05)(Df, Dm) * (Df ** -0.5)),
        }
    _B_in = _B_setup()

    return {
        "A_x": _A_in["x"],
        "A_wqkv": _A_in["wqkv"],
        "A_wo": _A_in["wo"],
        "B_x": _B_in["x"],
        "B_w_gate": _B_in["w_gate"],
        "B_w_up": _B_in["w_up"],
        "B_w_down": _B_in["w_down"],
    }

def reference(A_x, A_wqkv, A_wo, B_x, B_w_gate, B_w_up, B_w_down):
    def _A_ref(x, wqkv, wo):
        B, S, D = x.shape
        H = 32; Dh = D // H
        W, dil = 8, 2
        qkv = (lambda x, *d: x.transpose(*d))((x @ wqkv).reshape(B, S, 3, H, Dh), 2, 0, 3, 1, 4)
        q, k, v = qkv[0], qkv[1], qkv[2]
        scale = Dh ** -0.5
        pos = jnp.arange(S)
        off = jnp.arange(W) * dil
        idx = pos[:, None] - off[None, :]
        mask = idx >= 0
        idx_c = jnp.where(mask, idx, 0).reshape(-1)
        kg = k[:, :, idx_c, :].reshape(B, H, S, W, Dh)
        vg = v[:, :, idx_c, :].reshape(B, H, S, W, Dh)
        logits = jnp.einsum("bhsd,bhswd->bhsw", q, kg) * scale
        logits = jnp.where(mask[None, None, :, :], logits, -1e9)
        attn = _softmax(logits, axis=-1)
        o = jnp.einsum("bhsw,bhswd->bhsd", attn, vg)
        return (lambda x, *d: x.transpose(*d))(o, 0, 2, 1, 3).reshape(B, S, D) @ wo

    def _B_ref(x, w_gate, w_up, w_down):
        g = jnp.einsum("bsd,df->bsf", x, w_gate)
        u = jnp.einsum("bsd,df->bsf", x, w_up)
        h = _gelu(g) * u
        return jnp.einsum("bsf,fd->bsd", h, w_down)

    x = A_x
    xn = _layernorm(x, axis=-1)
    return x + _A_ref(xn, A_wqkv, A_wo) + _B_ref(xn, B_w_gate, B_w_up, B_w_down)
```

```python
import functools
import numpy as np
import jax
import jax.numpy as jnp
import jax.experimental.pallas as pl
import jax.experimental.pallas.tpu as pltpu

S, D, DF = 2048, 1024, 3584
H, DH, W, DIL = 32, 32, 8, 2
HALO = 16
TH = S // 2
KH = D // 2
BF, F32 = jnp.bfloat16, jnp.float32
STR = 33
ORDER = (2, 4, 1, 3, 0, 6, 5)


def _dot(a, b):
    return jnp.dot(a, b, preferred_element_type=F32)


def _a_ops(a11, a12, a21, a22):
    return [t.astype(BF) for t in (a11 + a22, a21 + a22, a11, a22, a11 + a12, a21 - a11, a12 - a22)]


def _b_ops(b11, b12, b21, b22):
    f = lambda t: t.astype(F32)
    return [lambda: (f(b11()) + f(b22())).astype(BF),
            b11,
            lambda: (f(b12()) - f(b22())).astype(BF),
            lambda: (f(b21()) - f(b11())).astype(BF),
            b22,
            lambda: (f(b11()) + f(b12())).astype(BF),
            lambda: (f(b21()) + f(b22())).astype(BF)]


def _strassen(prod, emit):
    m3, m5 = prod(2), prod(4)
    emit(1, m3 + m5)
    m2, m4 = prod(1), prod(3)
    emit(2, m2 + m4)
    m1, m7 = prod(0), prod(6)
    emit(0, (m4 - m5) + m1 + m7)
    m6 = prod(5)
    emit(3, (m3 - m2) + m1 + m6)


def _quadrants(ref, r0, k, c0, n):
    return (lambda: ref[r0:r0 + k, c0:c0 + n], lambda: ref[r0:r0 + k, c0 + n:c0 + 2 * n],
            lambda: ref[r0 + k:r0 + 2 * k, c0:c0 + n], lambda: ref[r0 + k:r0 + 2 * k, c0 + n:c0 + 2 * n])


def _gelu_mul(g, u):
    c = float(np.sqrt(2.0 / np.pi))
    z = g * (c + (c * 0.044715) * (g * g))
    return ((0.5 * g) * u) * (1.0 + jnp.tanh(z))


def make(chunks=(512,) * 7, blocks=(128, 128, 128, 256, 384), wo_at=None, NO=128, LNR=16, PR=64, att_w=(1, 1, 1, 1, 1), att_n=13, n_units=64, flags=None,
         vmem_mb=125, scopes=False, fold=True):
    DFU = sum(chunks)
    c_off = [sum(chunks[:i]) for i in range(len(chunks) + 1)]
    b_off = [sum(blocks[:i]) for i in range(len(blocks) + 1)]
    nb = len(blocks)

    def scope(name):
        import contextlib
        return jax.named_scope(name) if scopes else contextlib.nullcontext()

    def kernel(x_hbm, wqkv_hbm, wo_hbm, wg_hbm, wu_hbm, wd_hbm, out_hbm,
               x_s, xa_s, wqkv_s, qkv_s, wg_s, wu_s, wd_s, wo_s, wof_s, sems):
        sem_id = iter(range(sems.shape[0]))

        def copy(src, dst):
            return pltpu.make_async_copy(src, dst, sems.at[next(sem_id)])

        def cols(hbm, vmem, lo, hi):
            return copy(hbm.at[:, lo:hi], vmem.at[:, lo:hi])

        def rows(hbm, vmem, lo, hi):
            return copy(hbm.at[lo:hi, :], vmem.at[lo:hi, :])

        def start(cps):
            for cp in cps:
                cp.start()

        def wait(cps):
            for cp in cps:
                cp.wait()

        def ln(r, n):
            x = x_s[pl.ds(r, n), :].astype(F32)
            xc = x - jnp.mean(x, axis=-1, keepdims=True)
            var = jnp.mean(xc * xc, axis=-1, keepdims=True)
            return xc * jax.lax.rsqrt(var + 1e-5)

        def permute_cols(t, r, n):
            lane = jax.lax.broadcasted_iota(jnp.int32, (n // 2, 128), 1)
            tiles = []
            for k in range(8):
                w = pltpu.bitcast(wqkv_s[r:r + n, t * D + k * 128:t * D + (k + 1) * 128], jnp.uint32)
                src = (lane - 4 * k) & 127 if fold else lane
                idx = ((src & 3) << 5) | (src & 28) | (src >> 5)
                w = jnp.take_along_axis(w, idx, axis=1, mode="promise_in_bounds")
                tiles.append(w if (k == 0 or fold) else pltpu.roll(w, 4 * k, 1))
            xs = [tiles[(-k) % 8] for k in range(8)]
            for b in range(3):
                sel = (lane & (4 << b)) != 0
                xs = [jnp.where(sel, xs[(k - (1 << b)) % 8], xs[k]) for k in range(8)]
            for j in range(8):
                y = xs[j] if j == 0 else pltpu.roll(xs[j], 128 - 4 * j, 1)
                wqkv_s[r:r + n, t * D + j * 128:t * D + (j + 1) * 128] = pltpu.bitcast(y, BF)

        def permute_wo(j):
            cs = slice(j * 128, (j + 1) * 128)
            for h in range(H):
                wof_s[j % 4, h * STR:h * STR + DH, :] = wo_s[h * DH:(h + 1) * DH, cs].astype(F32)
            for d in range(DH):
                wo_s[d * H:(d + 1) * H, cs] = wof_s[j % 4, pl.ds(d, H, stride=STR), :].astype(BF)

        c_exp = float(DH ** -0.5 * np.log2(np.e))
        neg = float(-1e9 / DH ** -0.5)

        def window(t, j, r, w):
            return qkv_s[t, j, HALO + r - DIL * w:HALO + r - DIL * w + 16, :]

        def attn_probs(r):
            q = [window(0, j, r, 0) for j in range(8)]
            logits = []
            for w in range(W):
                pr = [q[j] * window(1, j, r, w) for j in range(8)]
                t = ((pr[0] + pr[1]) + (pr[2] + pr[3])) + ((pr[4] + pr[5]) + (pr[6] + pr[7]))
                t = t + pltpu.roll(t, 64, 1)
                t = t + pltpu.roll(t, 32, 1)
                if r < DIL * w:
                    pos = r + jax.lax.broadcasted_iota(jnp.int32, (16, 128), 0)
                    t = jnp.where(pos >= DIL * w, t, neg)
                logits.append(t)
            mx = functools.reduce(jnp.maximum, logits)
            e = [jnp.exp2((t - mx) * c_exp) for t in logits]
            inv = 1.0 / functools.reduce(jnp.add, e)
            return [t * inv for t in e]

        def attn_out(p, r, j):
            return functools.reduce(jnp.add, [p[w] * window(2, j, r, w) for w in range(W)])

        def attn_unit(r):
            pt, pb = attn_probs(r), attn_probs(TH + r)
            for j in range(4):
                ops = _a_ops(attn_out(pt, r, j), attn_out(pt, r, j + 4),
                             attn_out(pb, TH + r, j), attn_out(pb, TH + r, j + 4))
                for p, a in enumerate(ops):
                    wqkv_s[r:r + 16, p * KH + j * 128:p * KH + (j + 1) * 128] = a

        riders = []

        def mm(a, b):
            v = _dot(a, b)
            for f in (riders.pop(0) if riders else ()):
                f()
            return v

        def ride(work, n):
            assert not riders
            riders.extend(work[i * len(work) // n:(i + 1) * len(work) // n] for i in range(n))

        def up_proj(w_s, c):
            bops = _b_ops(*_quadrants(w_s, 0, KH, c_off[c], chunks[c] // 2))
            q = {}
            _strassen(lambda p: mm(xa_s[p], bops[p]()), q.__setitem__)
            return [q[i] for i in range(4)]

        def down(c, g, u, acc):
            ha = _a_ops(*[_gelu_mul(a, b) for a, b in zip(g, u)])
            dops = _b_ops(*_quadrants(wd_s, c_off[c], chunks[c] // 2, 0, KH))
            out = {}
            for p in ORDER:
                v = mm(ha[p], dops[p]())
                out[p] = v if acc is None else acc[p] + v
            return out

        def project(t):
            def emit(i, quad):
                row0, j0 = (i // 2) * TH, (i % 2) * 4
                for j in range(4):
                    blk = quad[:, j * 128:(j + 1) * 128]
                    qkv_s[t, j0 + j, HALO + row0:HALO + row0 + TH, :] = blk
                    if row0 == 0 and t > 0:
                        qkv_s[t, j0 + j, 0:HALO, :] = jnp.broadcast_to(blk[0:1, :], (HALO, 128))
            bops = _b_ops(*_quadrants(wqkv_s, 0, KH, t * D, KH))
            _strassen(lambda p: mm(xa_s[p], bops[p]()), emit)

        def ffn_copies(lo, hi):
            return [cols(wg_hbm, wg_s, lo, hi), cols(wu_hbm, wu_s, lo, hi), rows(wd_hbm, wd_s, lo, hi)]

        cp_x = [[rows(x_hbm, x_s, t + b_off[b], t + b_off[b + 1]) for t in (0, TH)] for b in range(nb)]
        grp0 = ffn_copies(0, c_off[1])
        grp1 = ffn_copies(c_off[1], c_off[2]) + [copy(wqkv_hbm, wqkv_s.at[:, 0:3 * D]), copy(wo_hbm, wo_s)]
        grp2 = ffn_copies(c_off[2], DFU)

        def ln_block(b):
            for r in range(b_off[b], b_off[b + 1], LNR):
                top, bot = ln(r, LNR), ln(TH + r, LNR)
                for p, a in enumerate(_a_ops(top[:, :KH], top[:, KH:], bot[:, :KH], bot[:, KH:])):
                    xa_s[p, r:r + LNR, :] = a

        with scope("c0"):
            start(cp_x[0] + grp0[:1] + sum(cp_x[1:], []) + grp0[1:] + grp1 + grp2)
            wait(cp_x[0])
            ln_block(0)
            wait(grp0[:1])
            gops = [(lambda v=f(): v) for f in _b_ops(*_quadrants(wg_s, 0, KH, 0, chunks[0] // 2))]
            parts = []
            for b in range(nb):
                if b + 1 < nb:
                    wait(cp_x[b + 1])
                    ln_block(b + 1)
                q = {}
                _strassen(lambda p: _dot(xa_s[p, b_off[b]:b_off[b + 1], :], gops[p]()), q.__setitem__)
                parts.append(q)
            g = [jnp.concatenate([q[i] for q in parts], axis=0) for i in range(4)]
            wait(grp0[1:])
            acc = down(0, g, up_proj(wu_s, 0), None)

        with scope("c1"):
            wait(grp1)
            work = [functools.partial(permute_cols, t, r, PR) for t in range(3) for r in range(0, D, PR)]
            ride(work, 14)
            g, u = up_proj(wg_s, 1), up_proj(wu_s, 1)
            acc = down(1, g, u, acc)

        with scope("main"):
            ride([functools.partial(permute_wo, j) for j in range(8)], 21)
            for t in range(3):
                project(t)

        with scope("ffn"):
            wait(grp2)
            units = [functools.partial(attn_unit, r) for r in range(0, TH, 16)][:n_units]
            share = [w / sum(att_w) for w in att_w]
            done = 0
            for n, c in enumerate(range(2, len(chunks))):
                upto = round(sum(share[:n + 1]) * len(units))
                if upto > done:
                    ride(units[done:upto], min(att_n, upto - done))
                done = upto
                g = up_proj(wg_s, c)
                if c == wo_at:
                    bops = _b_ops(*_quadrants(wo_s, 0, KH, 0, KH))
                    acc = {p: acc[p] + mm(wqkv_s[:, p * KH:(p + 1) * KH], bops[p]()) for p in ORDER}
                u = up_proj(wu_s, c)
                if c + 1 < len(chunks) or wo_at is None:
                    acc = down(c, g, u, acc)

            out_cps = []
            ha = _a_ops(*[_gelu_mul(a, b) for a, b in zip(g, u)])
            for j in range(KH // NO):
                lo, hi = slice(j * NO, (j + 1) * NO), slice(KH + j * NO, KH + (j + 1) * NO)
                if wo_at is None:
                    w_s, r0, k, lhs = wo_s, 0, KH, lambda p: wqkv_s[:, p * KH:(p + 1) * KH]
                else:
                    w_s, r0, k, lhs = wd_s, c_off[-2], chunks[-1] // 2, lambda p: ha[p]
                bops = _b_ops(lambda: w_s[r0:r0 + k, lo], lambda: w_s[r0:r0 + k, hi],
                              lambda: w_s[r0 + k:r0 + 2 * k, lo], lambda: w_s[r0 + k:r0 + 2 * k, hi])

                def emit(i, quad):
                    rs, cs = slice((i // 2) * TH, (i // 2 + 1) * TH), (lo, hi)[i % 2]
                    x_s[rs, cs] = (x_s[rs, cs].astype(F32) + quad).astype(BF)
                    out_cps.append(copy(x_s.at[rs, cs], out_hbm.at[rs, cs]))
                    out_cps[-1].start()
                _strassen(lambda p: acc[p][:, lo] + mm(lhs(p), bops[p]()), emit)
            wait(out_cps)

    def fn(A_x, A_wqkv, A_wo, B_x, B_w_gate, B_w_up, B_w_down):
        del B_x
        hbm = pl.BlockSpec(memory_space=pl.ANY)
        out = pl.pallas_call(
            kernel,
            in_specs=[hbm] * 6,
            out_specs=hbm,
            out_shape=jax.ShapeDtypeStruct((S, D), BF),
            scratch_shapes=[
                pltpu.VMEM((S, D), BF),
                pltpu.VMEM((7, TH, KH), BF),
                pltpu.VMEM((D, 7 * KH), BF),
                pltpu.VMEM((3, 8, HALO + S, 128), F32),
                pltpu.VMEM((D, DF), BF),
                pltpu.VMEM((D, DF), BF),
                pltpu.VMEM((DF, D), BF),
                pltpu.VMEM((D, D), BF),
                pltpu.VMEM((4, H * STR, 128), F32),
                pltpu.SemaphoreType.DMA((2 * nb + 11 + 16,)),
            ],
            compiler_params=pltpu.CompilerParams(vmem_limit_bytes=vmem_mb * 1024 * 1024, flags=flags),
        )(A_x.reshape(S, D), A_wqkv, A_wo, B_w_gate, B_w_up, B_w_down)
        return out.reshape(1, S, D)
    return fn


_impl = make(**dict(flags={'XLA_TPU_EVENLY_DISTRIBUTE_CRITICAL_NODES': True}))


@jax.jit
def pallas_parallel_sum__sliding_local_dilated__glu_gated_geglu__prompt_kernel(
    A_x: jax.Array,
    A_wqkv: jax.Array,
    A_wo: jax.Array,
    B_x: jax.Array,
    B_w_gate: jax.Array,
    B_w_up: jax.Array,
    B_w_down: jax.Array,
):
    return _impl(A_x, A_wqkv, A_wo, B_x, B_w_gate, B_w_up, B_w_down)
```

```python
import functools

import jax
import jax.experimental.pallas as pl
import jax.experimental.pallas.tpu as pltpu
import jax.numpy as jnp
import numpy as np

S, D, DF = 2048, 1024, 3584
H, DH, W, DIL = 32, 32, 8, 2
TH, KH = S // 2, D // 2
FC = 512
HALO = 16
STR = 33
LAG = 4
BF, F32, U32 = jnp.bfloat16, jnp.float32, jnp.uint32
ORDER = (4, 2, 1, 3, 0, 6, 5)


def _dot(a, b):
    return jnp.dot(a, b, preferred_element_type=F32)


def _left_ops(a11, a12, a21, a22):
    return [t.astype(BF) for t in (a11 + a22, a21 + a22, a11, a22, a11 + a12, a21 - a11, a12 - a22)]


def _right_ops(w, rows, cols):
    b11, b12, b21, b22 = (lambda r=r, c=c: w[r, c] for r in rows for c in cols)
    f = lambda t: t().astype(F32)
    return [lambda: (f(b11) + f(b22)).astype(BF), b11,
            lambda: (f(b12) - f(b22)).astype(BF),
            lambda: (f(b21) - f(b11)).astype(BF), b22,
            lambda: (f(b11) + f(b12)).astype(BF),
            lambda: (f(b21) + f(b22)).astype(BF)]


def _halves(start, size):
    return slice(start, start + size // 2), slice(start + size // 2, start + size)


def _strassen(product, emit):
    m5, m3 = product(4), product(2)
    emit(1, m3 + m5)
    m2, m4 = product(1), product(3)
    emit(2, m2 + m4)
    m1, m7 = product(0), product(6)
    emit(0, (m4 - m5) + m1 + m7)
    m6 = product(5)
    emit(3, (m3 - m2) + m1 + m6)


def _zero_after(values):
    tiles = []
    for v in values:
        v = pltpu.bitcast(v, U32)
        tiles += [v[r:r + 8, c:c + 128] for r in range(0, v.shape[0], 8) for c in range(0, v.shape[1], 128)]
    return (functools.reduce(jnp.bitwise_or, tiles) >> 31) >> 1


def _gelu_times(g, u):
    c = float(np.sqrt(2.0 / np.pi))
    z = g * (c + (c * 0.044715) * (g * g))
    return ((0.5 * g) * u) * (1.0 + jnp.tanh(z))


def _kernel(x_hbm, wqkv_hbm, wo_hbm, wg_hbm, wu_hbm, wd_hbm, out_hbm,
            x_s, wqkv_s, qkv_s, wg_s, wu_s, wd_s, wo_s, wot_s, sems):
    def copy(src, dst, index, group):
        return pltpu.make_async_copy(src.at[index], dst.at[index], sems.at[group])

    def x_rows(lo, hi, group):
        return [copy(x_hbm, x_s, (slice(t + lo, t + hi), slice(0, D)), group) for t in (0, TH)]

    def up_cols(hbm, vmem, lo, hi, group):
        return [copy(hbm, vmem, (slice(0, D), slice(lo, hi)), group)]

    def down_rows(lo, hi, group):
        return [copy(wd_hbm, wd_s, (slice(lo, hi), slice(0, D)), group)]

    def geglu_weights(lo, hi, group):
        return (up_cols(wg_hbm, wg_s, lo, hi, group) + up_cols(wu_hbm, wu_s, lo, hi, group)
                + down_rows(lo, hi, group))

    def wait(copies):
        for cp in copies:
            cp.wait()

    def pin(values):
        wot_s[7, 0:8, :] = pltpu.bitcast(_zero_after(values), F32)

    def layernorm(r):
        x = [x_s[r:r + 16, j * 128:(j + 1) * 128].astype(F32) for j in range(D // 128)]
        lane_sum = lambda t: jnp.broadcast_to(jnp.sum(t, axis=-1, keepdims=True), t.shape)
        mu = functools.reduce(jnp.add, x) * (128.0 / D)
        m2 = functools.reduce(jnp.add, [(t - mu) * (t - mu) for t in x])
        mean = lane_sum(mu) * (1.0 / 128)
        dm = mu - mean
        var = lane_sum(m2 + (D // 128) * (dm * dm)) * (1.0 / D)
        inv_std = jax.lax.rsqrt(var + 1e-5)
        return [(t - mean) * inv_std for t in x]

    xn_ops = {}

    def normalize(lo, hi):
        for r in range(lo, hi, 16):
            top, bot = layernorm(r), layernorm(TH + r)
            ops = [_left_ops(top[j], top[j + 4], bot[j], bot[j + 4]) for j in range(4)]
            xn_ops[r] = [jnp.concatenate(t, axis=1) for t in zip(*ops)]
        return [a for r in range(lo, hi, 16) for a in xn_ops[r]]

    def permute_columns(t, r):
        lane = jax.lax.broadcasted_iota(jnp.int32, (8, 128), 1)
        tiles = []
        for k in range(8):
            w = pltpu.bitcast(wqkv_s[r:r + 16, t * D + k * 128:t * D + (k + 1) * 128], U32)
            src = (lane - 4 * k) & 127
            idx = ((src & 3) << 5) | (src & 28) | (src >> 5)
            tiles.append(jnp.take_along_axis(w, idx, axis=1, mode="promise_in_bounds"))
        xs = [tiles[(-k) % 8] for k in range(8)]
        for b in range(3):
            sel = (lane & (4 << b)) != 0
            xs = [jnp.where(sel, xs[(k - (1 << b)) % 8], xs[k]) for k in range(8)]
        ys = [xs[j] if j == 0 else pltpu.roll(xs[j], 128 - 4 * j, 1) for j in range(8)]
        out = pltpu.bitcast(jnp.concatenate(ys, axis=1), BF)
        wqkv_s[r:r + 16, t * D:(t + 1) * D] = out
        return [out]

    def permuted_wo_tile(j):
        for h in range(H):
            wot_s[j, h * STR:h * STR + DH, :] = wo_s[h * DH:(h + 1) * DH, j * 128:(j + 1) * 128].astype(F32)
        return jnp.concatenate([wot_s[j, pl.ds(d, H, stride=STR), :].astype(BF) for d in range(DH)], axis=0)

    def window(t, j, r, w):
        return qkv_s[t, j, HALO + r - DIL * w:HALO + r - DIL * w + 16, :]

    def softmax_weights(r, after):
        scale = DH ** -0.5
        q = [window(0, j, r, 0) for j in range(8)]
        logits = []
        for w in range(W):
            pr = [q[j] * window(1, j, r, w) for j in range(8)]
            t = ((pr[0] + pr[1]) + (pr[2] + pr[3])) + ((pr[4] + pr[5]) + (pr[6] + pr[7]))
            if after is not None and w == 0:
                t = jnp.concatenate([pltpu.bitcast(pltpu.bitcast(t[0:8], U32) | after, F32), t[8:]], axis=0)
            t = t + pltpu.roll(t, 64, 1)
            t = t + pltpu.roll(t, 32, 1)
            if r < DIL * w:
                pos = r + jax.lax.broadcasted_iota(jnp.int32, (16, 128), 0)
                t = jnp.where(pos >= DIL * w, t, float(-1e9 / scale))
            logits.append(t)
        top = functools.reduce(jnp.maximum, logits)
        e = [jnp.exp2((t - top) * float(scale * np.log2(np.e))) for t in logits]
        inv = 1.0 / functools.reduce(jnp.add, e)
        return [t * inv for t in e]

    def attend(p, r, j):
        return functools.reduce(jnp.add, [p[w] * window(2, j, r, w) for w in range(W)])

    riders = []

    def paced(a, work):
        a = pltpu.bitcast(a, U32)
        step = a.shape[0] // 8 // len(work) * 8
        slabs = [a[:step // 16 * 8]] if step >= 16 else []
        for i, piece in enumerate(work):
            lo = step // 16 * 8 + i * step
            slab = a[lo:lo + step if i + 1 < len(work) else a.shape[0]]
            head = jnp.concatenate([slab[0:8, 0:128] | _zero_after(piece()), slab[0:8, 128:]], axis=1)
            slabs += [head, slab[8:]] if slab.shape[0] > 8 else [head]
        return pltpu.bitcast(jnp.concatenate(slabs, axis=0), BF)

    def matmul(a, b):
        if not riders:
            return _dot(a, b)
        n = 128 * 512 // b.shape[0]
        outs = []
        for c in range(0, b.shape[1], n):
            work = riders.pop(0) if riders else ()
            outs.append(_dot(paced(a, work) if work else a, b[:, c:c + n]))
        return jnp.concatenate(outs, axis=1)

    def xn_op(p, lo=0, hi=TH):
        return jnp.concatenate([xn_ops[r][p] for r in range(lo, hi, 16)], axis=0)

    def up_ops(w_s, c):
        return _right_ops(w_s, _halves(0, D), _halves(c * FC, FC))

    def down_ops(c):
        return _right_ops(wd_s, _halves(c * FC, FC), _halves(0, D))

    def up_proj(ops, lo=0, hi=TH, before=lambda p: None):
        quads = {}

        def product(p):
            before(p)
            return matmul(xn_op(p, lo, hi), ops[p]())
        _strassen(product, quads.__setitem__)
        return [quads[i] for i in range(4)]

    def hidden(g, u):
        return _left_ops(*[_gelu_times(a, b) for a, b in zip(g, u)])

    def down_proj(ops, h_ops, acc):
        out = {}
        for p in ORDER:
            v = matmul(h_ops[p], ops[p]())
            out[p] = v if acc is None else acc[p] + v
        return out

    def project(t, carry):
        def emit(i, quad):
            row0, j0 = (i // 2) * TH, (i % 2) * 4
            for j in range(4):
                blk = quad[:, j * 128:(j + 1) * 128]
                qkv_s[t, j0 + j, HALO + row0:HALO + row0 + TH, :] = blk
                if row0 == 0:
                    qkv_s[t, j0 + j, 0:HALO, :] = jnp.broadcast_to(blk[0:1, :], (HALO, 128))
        cols = (pl.ds(pl.multiple_of(t * D, D), KH), pl.ds(pl.multiple_of(t * D + KH, KH), KH))
        ops = _right_ops(wqkv_s, _halves(0, D), cols)
        _strassen(lambda p: matmul(xn_op(p), ops[p]()), emit)
        return carry

    edge = (0, 96, 192, 256, 448, 576, 704, TH)
    x0, x1 = x_rows(edge[0], edge[1], 0), x_rows(edge[1], edge[2], 1)
    gate_hi, gate_lo = up_cols(wg_hbm, wg_s, FC // 2, FC, 2), up_cols(wg_hbm, wg_s, 0, FC // 2, 3)
    second = up_cols(wu_hbm, wu_s, 0, FC, 4) + x_rows(edge[2], edge[3], 4)
    third = x_rows(edge[3], edge[5], 5)
    fourth = x_rows(edge[5], TH, 6) + down_rows(0, FC, 6)
    fifth = geglu_weights(FC, 2 * FC, 7) + [pltpu.make_async_copy(wqkv_hbm, wqkv_s, sems.at[7])]
    rest = [pltpu.make_async_copy(wo_hbm, wo_s, sems.at[8])] + geglu_weights(2 * FC, DF, 8)
    for cp in x0 + x1 + gate_hi + gate_lo + second + third + fourth + fifth + rest:
        cp.start()

    wait(x0)
    pin(normalize(edge[0], edge[1]))
    wait(x1)
    pin(normalize(edge[1], edge[2]))
    g_ops, u_ops, d_ops = ([functools.cache(f) for f in ops]
                           for ops in (up_ops(wg_s, 0), up_ops(wu_s, 0), down_ops(0)))
    block = lambda i: hidden(up_proj(g_ops, edge[i], edge[i + 1]), up_proj(u_ops, edge[i], edge[i + 1]))
    stack = lambda parts: [jnp.concatenate(t, axis=0) for t in zip(*parts)]
    wait(gate_hi)
    g = up_proj(g_ops, 0, edge[2], before=lambda p: wait(gate_lo) if p == ORDER[2] else None)
    wait(second)
    ahead = normalize(edge[2], edge[3])
    h = [hidden(g, up_proj(u_ops, 0, edge[2]))]
    pin(ahead)
    wait(third)
    ahead = normalize(edge[3], edge[5])
    h += [block(2), block(3)]
    pin(ahead[(edge[4] - edge[3]) // 16 * 7:])
    wait(fourth)
    normalize(edge[5], TH)
    h_late = [block(4)]
    acc0 = down_proj(d_ops, stack(h), None)
    h_late += [block(5), block(6)]
    acc1 = down_proj(d_ops, stack(h_late), None)
    acc = {p: jnp.concatenate([acc0[p], acc1[p]], axis=0) for p in ORDER}

    wait(fifth)
    work = [functools.partial(permute_columns, t, r) for t in range(3) for r in range(0, D, 16)]
    riders += [(), ()] + [work[i * len(work) // 40:(i + 1) * len(work) // 40] for i in range(40)]
    acc = down_proj(down_ops(1), hidden(up_proj(up_ops(wg_s, 1)), up_proj(up_ops(wu_s, 1))), acc)
    assert not riders
    jax.lax.fori_loop(0, 3, project, None)

    wait(rest)
    probs, done = {}, []
    for r in range(0, TH, 16):
        for t in (0, TH):
            probs[t + r] = softmax_weights(t + r, _zero_after(done[-LAG]) if len(done) >= LAG else None)
            done.append(probs[t + r])
    o_ops = {}
    for r in range(0, TH, 16):
        for j in range(4):
            o_ops[r, j] = _left_ops(attend(probs[r], r, j), attend(probs[r], r, j + 4),
                                    attend(probs[TH + r], TH + r, j), attend(probs[TH + r], TH + r, j + 4))
    for c in range(2, DF // FC):
        if c == 4:
            wo = jnp.concatenate([permuted_wo_tile(j) for j in range(8)], axis=1)
        acc = down_proj(down_ops(c), hidden(up_proj(up_ops(wg_s, c)), up_proj(up_ops(wu_s, c))), acc)

    def o_op(p):
        return jnp.concatenate([jnp.concatenate([o_ops[r, j][p] for j in range(4)], axis=1)
                                for r in range(0, TH, 16)], axis=0)

    stores = []
    for j in range(KH // 128):
        cols = (slice(j * 128, (j + 1) * 128), slice(KH + j * 128, KH + (j + 1) * 128))
        ops = _right_ops(wo, _halves(0, D), cols)

        def emit(i, quad):
            index = (slice((i // 2) * TH, (i // 2 + 1) * TH), cols[i % 2])
            x_s[index] = (x_s[index].astype(F32) + quad).astype(BF)
            stores.append(copy(x_s, out_hbm, index, 9))
            stores[-1].start()
        _strassen(lambda p: acc[p][:, cols[0]] + matmul(o_op(p), ops[p]()), emit)
    wait(stores)


@jax.jit
def pallas_parallel_sum__sliding_local_dilated__glu_gated_geglu__prompt_kernel(
    A_x: jax.Array,
    A_wqkv: jax.Array,
    A_wo: jax.Array,
    B_x: jax.Array,
    B_w_gate: jax.Array,
    B_w_up: jax.Array,
    B_w_down: jax.Array,
):
    del B_x
    hbm = pl.BlockSpec(memory_space=pl.ANY)
    out = pl.pallas_call(
        _kernel,
        in_specs=[hbm] * 6,
        out_specs=hbm,
        out_shape=jax.ShapeDtypeStruct((S, D), BF),
        scratch_shapes=[
            pltpu.VMEM((S, D), BF),
            pltpu.VMEM((D, 3 * D), BF),
            pltpu.VMEM((3, 8, HALO + S, 128), F32),
            pltpu.VMEM((D, DF), BF),
            pltpu.VMEM((D, DF), BF),
            pltpu.VMEM((DF, D), BF),
            pltpu.VMEM((D, D), BF),
            pltpu.VMEM((8, H * STR + DH, 128), F32),
            pltpu.SemaphoreType.DMA((10,)),
        ],
        compiler_params=pltpu.CompilerParams(
            vmem_limit_bytes=127 * 1024 * 1024,
            flags={"XLA_TPU_EVENLY_DISTRIBUTE_CRITICAL_NODES": True},
        ),
    )(A_x.reshape(S, D), A_wqkv, A_wo, B_w_gate, B_w_up, B_w_down)
    return out.reshape(1, S, D)
```

```python
import functools

import jax
import jax.experimental.pallas as pl
import jax.experimental.pallas.tpu as pltpu
import jax.numpy as jnp
import numpy as np

S, D, DF = 2048, 1024, 3584
H, DH, W, DIL = 32, 32, 8, 2
TH, KH = S // 2, D // 2
FC = 512
HALO = 16
STR = 33
LAG = 4
BF, F32, U32 = jnp.bfloat16, jnp.float32, jnp.uint32
ORDER = (4, 2, 1, 3, 0, 6, 5)


def _dot(a, b):
    return jnp.dot(a, b, preferred_element_type=F32)


def _left_ops(a11, a12, a21, a22):
    return [t.astype(BF) for t in (a11 + a22, a21 + a22, a11, a22, a11 + a12, a21 - a11, a12 - a22)]


def _right_ops(w, rows, cols):
    b11, b12, b21, b22 = (lambda r=r, c=c: w[r, c] for r in rows for c in cols)
    f = lambda t: t().astype(F32)
    return [lambda: (f(b11) + f(b22)).astype(BF), b11,
            lambda: (f(b12) - f(b22)).astype(BF),
            lambda: (f(b21) - f(b11)).astype(BF), b22,
            lambda: (f(b11) + f(b12)).astype(BF),
            lambda: (f(b21) + f(b22)).astype(BF)]


def _halves(start, size):
    return slice(start, start + size // 2), slice(start + size // 2, start + size)


def _strassen(product, emit):
    m5, m3 = product(4), product(2)
    emit(1, m3 + m5)
    m2, m4 = product(1), product(3)
    emit(2, m2 + m4)
    m1, m7 = product(0), product(6)
    emit(0, (m4 - m5) + m1 + m7)
    m6 = product(5)
    emit(3, (m3 - m2) + m1 + m6)


def _zero_after(values):
    tiles = []
    for v in values:
        v = pltpu.bitcast(v, U32)
        tiles += [v[r:r + 8, c:c + 128] for r in range(0, v.shape[0], 8) for c in range(0, v.shape[1], 128)]
    return (functools.reduce(jnp.bitwise_or, tiles) >> 31) >> 1


def _gelu_times(g, u):
    c = float(np.sqrt(2.0 / np.pi))
    z = g * (c + (c * 0.044715) * (g * g))
    return ((0.5 * g) * u) * (1.0 + jnp.tanh(z))


def _kernel(x_hbm, wqkv_hbm, wo_hbm, wg_hbm, wu_hbm, wd_hbm, out_hbm,
            x_s, wqkv_s, qkv_s, wg_s, wu_s, wd_s, wo_s, wot_s, sems):
    def copy(src, dst, index, group):
        return pltpu.make_async_copy(src.at[index], dst.at[index], sems.at[group])

    def x_rows(lo, hi, group):
        return [copy(x_hbm, x_s, (slice(t + lo, t + hi), slice(0, D)), group) for t in (0, TH)]

    def up_cols(hbm, vmem, lo, hi, group):
        return [copy(hbm, vmem, (slice(0, D), slice(lo, hi)), group)]

    def down_rows(lo, hi, group):
        return [copy(wd_hbm, wd_s, (slice(lo, hi), slice(0, D)), group)]

    def geglu_weights(lo, hi, group):
        return (up_cols(wg_hbm, wg_s, lo, hi, group) + up_cols(wu_hbm, wu_s, lo, hi, group)
                + down_rows(lo, hi, group))

    def wait(copies):
        for cp in copies:
            cp.wait()

    def pin(values):
        wot_s[7, 0:8, :] = pltpu.bitcast(_zero_after(values), F32)

    def layernorm(r):
        x = [x_s[r:r + 16, j * 128:(j + 1) * 128].astype(F32) for j in range(D // 128)]
        lane_sum = lambda t: jnp.broadcast_to(jnp.sum(t, axis=-1, keepdims=True), t.shape)
        mu = functools.reduce(jnp.add, x) * (128.0 / D)
        m2 = functools.reduce(jnp.add, [(t - mu) * (t - mu) for t in x])
        mean = lane_sum(mu) * (1.0 / 128)
        dm = mu - mean
        var = lane_sum(m2 + (D // 128) * (dm * dm)) * (1.0 / D)
        inv_std = jax.lax.rsqrt(var + 1e-5)
        return [(t - mean) * inv_std for t in x]

    xn_ops = {}

    def normalize(lo, hi):
        for r in range(lo, hi, 16):
            top, bot = layernorm(r), layernorm(TH + r)
            ops = [_left_ops(top[j], top[j + 4], bot[j], bot[j + 4]) for j in range(4)]
            xn_ops[r] = [jnp.concatenate(t, axis=1) for t in zip(*ops)]
        return [a for r in range(lo, hi, 16) for a in xn_ops[r]]

    def permute_columns(t, r):
        lane = jax.lax.broadcasted_iota(jnp.int32, (8, 128), 1)
        tiles = []
        for k in range(8):
            w = pltpu.bitcast(wqkv_s[r:r + 16, t * D + k * 128:t * D + (k + 1) * 128], U32)
            src = (lane - 4 * k) & 127
            idx = ((src & 3) << 5) | (src & 28) | (src >> 5)
            tiles.append(jnp.take_along_axis(w, idx, axis=1, mode="promise_in_bounds"))
        xs = [tiles[(-k) % 8] for k in range(8)]
        for b in range(3):
            sel = (lane & (4 << b)) != 0
            xs = [jnp.where(sel, xs[(k - (1 << b)) % 8], xs[k]) for k in range(8)]
        ys = [xs[j] if j == 0 else pltpu.roll(xs[j], 128 - 4 * j, 1) for j in range(8)]
        out = pltpu.bitcast(jnp.concatenate(ys, axis=1), BF)
        wqkv_s[r:r + 16, t * D:(t + 1) * D] = out
        return [out]

    def permuted_wo_tile(j):
        for h in range(H):
            wot_s[j, h * STR:h * STR + DH, :] = wo_s[h * DH:(h + 1) * DH, j * 128:(j + 1) * 128].astype(F32)
        return jnp.concatenate([wot_s[j, pl.ds(d, H, stride=STR), :].astype(BF) for d in range(DH)], axis=0)

    def window(t, j, r, w):
        return qkv_s[t, j, HALO + r - DIL * w:HALO + r - DIL * w + 16, :]

    def softmax_weights(r, after):
        scale = DH ** -0.5
        q = [window(0, j, r, 0) for j in range(8)]
        logits = []
        for w in range(W):
            pr = [q[j] * window(1, j, r, w) for j in range(8)]
            t = ((pr[0] + pr[1]) + (pr[2] + pr[3])) + ((pr[4] + pr[5]) + (pr[6] + pr[7]))
            if after is not None and w == 0:
                t = jnp.concatenate([pltpu.bitcast(pltpu.bitcast(t[0:8], U32) | after, F32), t[8:]], axis=0)
            t = t + pltpu.roll(t, 64, 1)
            t = t + pltpu.roll(t, 32, 1)
            if r < DIL * w:
                pos = r + jax.lax.broadcasted_iota(jnp.int32, (16, 128), 0)
                t = jnp.where(pos >= DIL * w, t, float(-1e9 / scale))
            logits.append(t)
        top = functools.reduce(jnp.maximum, logits)
        e = [jnp.exp2((t - top) * float(scale * np.log2(np.e))) for t in logits]
        inv = 1.0 / functools.reduce(jnp.add, e)
        return [t * inv for t in e]

    def attend(p, r, j):
        return functools.reduce(jnp.add, [p[w] * window(2, j, r, w) for w in range(W)])

    riders = []

    def paced(a, work):
        a = pltpu.bitcast(a, U32)
        step = a.shape[0] // 8 // len(work) * 8
        slabs = [a[:step // 16 * 8]] if step >= 16 else []
        for i, piece in enumerate(work):
            lo = step // 16 * 8 + i * step
            slab = a[lo:lo + step if i + 1 < len(work) else a.shape[0]]
            head = jnp.concatenate([slab[0:8, 0:128] | _zero_after(piece()), slab[0:8, 128:]], axis=1)
            slabs += [head, slab[8:]] if slab.shape[0] > 8 else [head]
        return pltpu.bitcast(jnp.concatenate(slabs, axis=0), BF)

    def matmul(a, b):
        if not riders:
            return _dot(a, b)
        n = 128 * 512 // b.shape[0]
        outs = []
        for c in range(0, b.shape[1], n):
            work = riders.pop(0) if riders else ()
            outs.append(_dot(paced(a, work) if work else a, b[:, c:c + n]))
        return jnp.concatenate(outs, axis=1)

    def xn_op(p, lo=0, hi=TH):
        return jnp.concatenate([xn_ops[r][p] for r in range(lo, hi, 16)], axis=0)

    def up_ops(w_s, c):
        return _right_ops(w_s, _halves(0, D), _halves(c * FC, FC))

    def down_ops(c):
        return _right_ops(wd_s, _halves(c * FC, FC), _halves(0, D))

    def up_proj(ops, lo=0, hi=TH, before=lambda p: None):
        quads = {}

        def product(p):
            before(p)
            return matmul(xn_op(p, lo, hi), ops[p]())
        _strassen(product, quads.__setitem__)
        return [quads[i] for i in range(4)]

    def hidden(g, u):
        return _left_ops(*[_gelu_times(a, b) for a, b in zip(g, u)])

    def down_proj(ops, h_ops, acc):
        out = {}
        for p in ORDER:
            v = matmul(h_ops[p], ops[p]())
            out[p] = v if acc is None else acc[p] + v
        return out

    def project(t, carry):
        def emit(i, quad):
            row0, j0 = (i // 2) * TH, (i % 2) * 4
            for j in range(4):
                blk = quad[:, j * 128:(j + 1) * 128]
                qkv_s[t, j0 + j, HALO + row0:HALO + row0 + TH, :] = blk
                if row0 == 0:
                    qkv_s[t, j0 + j, 0:HALO, :] = jnp.broadcast_to(blk[0:1, :], (HALO, 128))
        cols = (pl.ds(pl.multiple_of(t * D, D), KH), pl.ds(pl.multiple_of(t * D + KH, KH), KH))
        ops = _right_ops(wqkv_s, _halves(0, D), cols)
        _strassen(lambda p: matmul(xn_op(p), ops[p]()), emit)
        return carry

    edge = (0, 96, 192, 256, 448, 576, 704, TH)
    x0, x1 = x_rows(edge[0], edge[1], 0), x_rows(edge[1], edge[2], 1)
    gate_hi, gate_lo = up_cols(wg_hbm, wg_s, FC // 2, FC, 2), up_cols(wg_hbm, wg_s, 0, FC // 2, 3)
    second = up_cols(wu_hbm, wu_s, 0, FC, 4) + x_rows(edge[2], edge[3], 4)
    third = x_rows(edge[3], edge[5], 5)
    fourth = x_rows(edge[5], TH, 6) + down_rows(0, FC, 6)
    fifth = geglu_weights(FC, 2 * FC, 7) + [pltpu.make_async_copy(wqkv_hbm, wqkv_s, sems.at[7])]
    rest = [pltpu.make_async_copy(wo_hbm, wo_s, sems.at[8])] + geglu_weights(2 * FC, DF, 8)
    for cp in x0 + x1 + gate_hi + gate_lo + second + third + fourth + fifth + rest:
        cp.start()

    wait(x0)
    pin(normalize(edge[0], edge[1]))
    wait(x1)
    pin(normalize(edge[1], edge[2]))
    g_ops, u_ops, d_ops = ([functools.cache(f) for f in ops]
                           for ops in (up_ops(wg_s, 0), up_ops(wu_s, 0), down_ops(0)))
    block = lambda i: hidden(up_proj(g_ops, edge[i], edge[i + 1]), up_proj(u_ops, edge[i], edge[i + 1]))
    stack = lambda parts: [jnp.concatenate(t, axis=0) for t in zip(*parts)]
    wait(gate_hi)
    g = up_proj(g_ops, 0, edge[2], before=lambda p: wait(gate_lo) if p == ORDER[2] else None)
    wait(second)
    ahead = normalize(edge[2], edge[3])
    h = [hidden(g, up_proj(u_ops, 0, edge[2]))]
    pin(ahead)
    wait(third)
    ahead = normalize(edge[3], edge[5])
    h += [block(2), block(3)]
    pin(ahead[(edge[4] - edge[3]) // 16 * 7:])
    wait(fourth)
    normalize(edge[5], TH)
    h_late = [block(4)]
    acc0 = down_proj(d_ops, stack(h), None)
    h_late += [block(5), block(6)]
    acc1 = down_proj(d_ops, stack(h_late), None)
    acc = {p: jnp.concatenate([acc0[p], acc1[p]], axis=0) for p in ORDER}

    wait(fifth)
    work = [functools.partial(permute_columns, t, r) for t in range(3) for r in range(0, D, 16)]
    riders += [(), ()] + [work[i * len(work) // 40:(i + 1) * len(work) // 40] for i in range(40)]
    acc = down_proj(down_ops(1), hidden(up_proj(up_ops(wg_s, 1)), up_proj(up_ops(wu_s, 1))), acc)
    assert not riders
    jax.lax.fori_loop(0, 3, project, None)

    wait(rest)
    probs, done = {}, []
    for r in range(0, TH, 16):
        for t in (0, TH):
            probs[t + r] = softmax_weights(t + r, _zero_after(done[-LAG]) if len(done) >= LAG else None)
            done.append(probs[t + r])
    o_ops = {}
    for r in range(0, TH, 16):
        for j in range(4):
            o_ops[r, j] = _left_ops(attend(probs[r], r, j), attend(probs[r], r, j + 4),
                                    attend(probs[TH + r], TH + r, j), attend(probs[TH + r], TH + r, j + 4))
    for c in range(2, DF // FC):
        if c == 4:
            wo = jnp.concatenate([permuted_wo_tile(j) for j in range(8)], axis=1)
        acc = down_proj(down_ops(c), hidden(up_proj(up_ops(wg_s, c)), up_proj(up_ops(wu_s, c))), acc)

    def o_op(p):
        return jnp.concatenate([jnp.concatenate([o_ops[r, j][p] for j in range(4)], axis=1)
                                for r in range(0, TH, 16)], axis=0)

    stores = []
    for j in range(KH // 128):
        cols = (slice(j * 128, (j + 1) * 128), slice(KH + j * 128, KH + (j + 1) * 128))
        ops = _right_ops(wo, _halves(0, D), cols)

        def emit(i, quad):
            n = TH // 8 if (j, i) == (KH // 128 - 1, 3) else TH
            for r in range(0, TH, n):
                index = (slice((i // 2) * TH + r, (i // 2) * TH + r + n), cols[i % 2])
                x_s[index] = (x_s[index].astype(F32) + quad[r:r + n]).astype(BF)
                stores.append(copy(x_s, out_hbm, index, 9))
                stores[-1].start()
        _strassen(lambda p: acc[p][:, cols[0]] + matmul(o_op(p), ops[p]()), emit)
    wait(stores)


@jax.jit
def pallas_parallel_sum__sliding_local_dilated__glu_gated_geglu__prompt_kernel(
    A_x: jax.Array,
    A_wqkv: jax.Array,
    A_wo: jax.Array,
    B_x: jax.Array,
    B_w_gate: jax.Array,
    B_w_up: jax.Array,
    B_w_down: jax.Array,
):
    del B_x
    hbm = pl.BlockSpec(memory_space=pl.ANY)
    out = pl.pallas_call(
        _kernel,
        in_specs=[hbm] * 6,
        out_specs=hbm,
        out_shape=jax.ShapeDtypeStruct((S, D), BF),
        scratch_shapes=[
            pltpu.VMEM((S, D), BF),
            pltpu.VMEM((D, 3 * D), BF),
            pltpu.VMEM((3, 8, HALO + S, 128), F32),
            pltpu.VMEM((D, DF), BF),
            pltpu.VMEM((D, DF), BF),
            pltpu.VMEM((DF, D), BF),
            pltpu.VMEM((D, D), BF),
            pltpu.VMEM((8, H * STR + DH, 128), F32),
            pltpu.SemaphoreType.DMA((10,)),
        ],
        compiler_params=pltpu.CompilerParams(
            vmem_limit_bytes=127 * 1024 * 1024,
            flags={"XLA_TPU_EVENLY_DISTRIBUTE_CRITICAL_NODES": True},
        ),
    )(A_x.reshape(S, D), A_wqkv, A_wo, B_w_gate, B_w_up, B_w_down)
    return out.reshape(1, S, D)
```

```python
import functools
import numpy as np
import jax
import jax.numpy as jnp
import jax.experimental.pallas as pl
import jax.experimental.pallas.tpu as pltpu

S, D, DF = 2048, 1024, 3584
H, DH, W, DIL = 32, 32, 8, 2
HALO = 16
TH = S // 2
KH = D // 2
BF, F32, U32 = jnp.bfloat16, jnp.float32, jnp.uint32
STR = 33
ORDER = (4, 2, 1, 3, 0, 6, 5)


def _dot(a, b):
    return jnp.dot(a, b, preferred_element_type=F32)


def _a_ops(a11, a12, a21, a22):
    return [t.astype(BF) for t in (a11 + a22, a21 + a22, a11, a22, a11 + a12, a21 - a11, a12 - a22)]


def _b_ops(b11, b12, b21, b22):
    f = lambda t: t.astype(F32)
    return [lambda: (f(b11()) + f(b22())).astype(BF),
            b11,
            lambda: (f(b12()) - f(b22())).astype(BF),
            lambda: (f(b21()) - f(b11())).astype(BF),
            b22,
            lambda: (f(b11()) + f(b12())).astype(BF),
            lambda: (f(b21()) + f(b22())).astype(BF)]


def _once(fs):
    vals = {}

    def get(i):
        if i not in vals:
            vals[i] = fs[i]()
        return vals[i]
    return [functools.partial(get, i) for i in range(len(fs))]


def _zero_after(vals):
    tiles = []
    for v in vals:
        v = pltpu.bitcast(v, U32)
        tiles += [v[r:r + 8, c:c + 128] for r in range(0, v.shape[0], 8) for c in range(0, v.shape[1], 128)]
    return (functools.reduce(jnp.bitwise_or, tiles) >> 31) >> 1


def _strassen(prod, emit):
    m5, m3 = prod(4), prod(2)
    emit(1, m3 + m5)
    m2, m4 = prod(1), prod(3)
    emit(2, m2 + m4)
    m1, m7 = prod(0), prod(6)
    emit(0, (m4 - m5) + m1 + m7)
    m6 = prod(5)
    emit(3, (m3 - m2) + m1 + m6)


def _quadrants(ref, r0, k, c0, n):
    return (lambda: ref[r0:r0 + k, c0:c0 + n], lambda: ref[r0:r0 + k, c0 + n:c0 + 2 * n],
            lambda: ref[r0 + k:r0 + 2 * k, c0:c0 + n], lambda: ref[r0 + k:r0 + 2 * k, c0 + n:c0 + 2 * n])


def _gelu_mul(g, u):
    c = float(np.sqrt(2.0 / np.pi))
    z = g * (c + (c * 0.044715) * (g * g))
    return ((0.5 * g) * u) * (1.0 + jnp.tanh(z))


def make(chunks=(512,) * 7, blocks=(256, 128, 128, 128, 384), RB=128, wo_at=None, NO=128, PR=64,
         n_units=64, flags=None, stop=None, vmem_mb=127, scopes=False, pv_n=40, ln_skip=2, ln_n=0, ln_n2=0, perm_n=40, pv_from=4, h_n=16, pin1=True):
    DFU = sum(chunks)
    c_off = [sum(chunks[:i]) for i in range(len(chunks) + 1)]
    b_off = [sum(blocks[:i]) for i in range(len(blocks) + 1)]
    nb = len(blocks)

    def scope(name):
        import contextlib
        return jax.named_scope(name) if scopes else contextlib.nullcontext()

    def kernel(x_hbm, wqkv_hbm, wo_hbm, wg_hbm, wu_hbm, wd_hbm, out_hbm,
               x_s, wqkv_s, qkv_s, wg_s, wu_s, wd_s, wo_s, wof_s, sems):
        sem_id = iter(range(sems.shape[0]))

        def copy(src, dst):
            return pltpu.make_async_copy(src, dst, sems.at[next(sem_id)])

        def cols(hbm, vmem, lo, hi):
            return copy(hbm.at[:, lo:hi], vmem.at[:, lo:hi])

        def rows(hbm, vmem, lo, hi):
            return copy(hbm.at[lo:hi, :], vmem.at[lo:hi, :])

        def start(cps):
            for cp in cps:
                cp.start()

        def wait(cps):
            for cp in cps:
                cp.wait()

        def ln(r, n):
            x = [x_s[r:r + n, j * 128:(j + 1) * 128].astype(F32) for j in range(D // 128)]
            lanesum = lambda t: jnp.broadcast_to(jnp.sum(t, axis=-1, keepdims=True), t.shape)
            mu = functools.reduce(jnp.add, x) * (128.0 / D)
            m2 = functools.reduce(jnp.add, [(t - mu) * (t - mu) for t in x])
            mean = lanesum(mu) * (1.0 / 128)
            dm = mu - mean
            var = lanesum(m2 + (D // 128) * (dm * dm)) * (1.0 / D)
            rs = jax.lax.rsqrt(var + 1e-5)
            return [(t - mean) * rs for t in x]

        xa = {}

        def ln_unit(r):
            top, bot = ln(r, 16), ln(TH + r, 16)
            ops = [_a_ops(top[j], top[j + 4], bot[j], bot[j + 4]) for j in range(4)]
            xa[r] = [jnp.concatenate(t, axis=1) for t in zip(*ops)]
            return xa[r]

        wp = {}

        def permute_cols(t, r):
            lane = jax.lax.broadcasted_iota(jnp.int32, (8, 128), 1)
            tiles = []
            for k in range(8):
                w = pltpu.bitcast(wqkv_s[r:r + 16, t * D + k * 128:t * D + (k + 1) * 128], U32)
                src = (lane - 4 * k) & 127
                idx = ((src & 3) << 5) | (src & 28) | (src >> 5)
                tiles.append(jnp.take_along_axis(w, idx, axis=1, mode="promise_in_bounds"))
            xs = [tiles[(-k) % 8] for k in range(8)]
            for b in range(3):
                sel = (lane & (4 << b)) != 0
                xs = [jnp.where(sel, xs[(k - (1 << b)) % 8], xs[k]) for k in range(8)]
            ys = [xs[j] if j == 0 else pltpu.roll(xs[j], 128 - 4 * j, 1) for j in range(8)]
            wp[t, r] = pltpu.bitcast(jnp.concatenate(ys, axis=1), BF)
            return [wp[t, r]]

        wop = {}

        def permute_wo(j):
            for h in range(H):
                wof_s[j, h * STR:h * STR + DH, :] = wo_s[h * DH:(h + 1) * DH, j * 128:(j + 1) * 128].astype(F32)
            wop[j] = jnp.concatenate([wof_s[j, pl.ds(d, H, stride=STR), :].astype(BF) for d in range(DH)], axis=0)
            return [wop[j]]

        c_exp = float(DH ** -0.5 * np.log2(np.e))
        neg = float(-1e9 / DH ** -0.5)

        def window(t, j, r, w):
            return qkv_s[t, j, HALO + r - DIL * w:HALO + r - DIL * w + 16, :]

        probs = {}

        def attn_probs(r):
            q = [window(0, j, r, 0) for j in range(8)]
            logits = []
            for w in range(W):
                pr = [q[j] * window(1, j, r, w) for j in range(8)]
                t = ((pr[0] + pr[1]) + (pr[2] + pr[3])) + ((pr[4] + pr[5]) + (pr[6] + pr[7]))
                t = t + pltpu.roll(t, 64, 1)
                t = t + pltpu.roll(t, 32, 1)
                if r < DIL * w:
                    pos = r + jax.lax.broadcasted_iota(jnp.int32, (16, 128), 0)
                    t = jnp.where(pos >= DIL * w, t, neg)
                logits.append(t)
            mx = functools.reduce(jnp.maximum, logits)
            e = [jnp.exp2((t - mx) * c_exp) for t in logits]
            inv = 1.0 / functools.reduce(jnp.add, e)
            probs[r] = [t * inv for t in e]
            return [inv]

        oa = {}

        def attn_mix(r, j):
            out = lambda r0, jj: functools.reduce(jnp.add, [probs[r0][w] * window(2, jj, r0, w) for w in range(W)])
            oa[r, j] = _a_ops(out(r, j), out(r, j + 4), out(TH + r, j), out(TH + r, j + 4))
            return oa[r, j]

        def get_xa(p, lo=0, hi=TH):
            return jnp.concatenate([xa[r][p] for r in range(lo, hi, 16)], axis=0)

        def get_oa(p):
            return jnp.concatenate([jnp.concatenate([oa[r % (16 * n_units), j][p] for j in range(4)], axis=1)
                                    for r in range(0, TH, 16)], axis=0)

        riders = []

        def paced(a, work):
            a = pltpu.bitcast(a, U32)
            step = a.shape[0] // 8 // len(work) * 8
            slabs = [a[:step // 16 * 8]] if step >= 16 else []
            for i, f in enumerate(work):
                lo = step // 16 * 8 + i * step
                slab = a[lo:lo + step if i + 1 < len(work) else a.shape[0]]
                head = jnp.concatenate([slab[0:8, 0:128] | _zero_after(f()), slab[0:8, 128:]], axis=1)
                slabs += [head, slab[8:]] if slab.shape[0] > 8 else [head]
            return pltpu.bitcast(jnp.concatenate(slabs, axis=0), BF)

        def mm(a, b):
            if not riders:
                return _dot(a, b)
            n = 128 * 512 // b.shape[0]
            outs = []
            for c in range(0, b.shape[1], n):
                work = riders.pop(0) if riders else ()
                outs.append(_dot(paced(a, work) if work else a, b[:, c:c + n]))
            return jnp.concatenate(outs, axis=1)

        def ride(work, n, skip=0):
            assert not riders
            if n == 0:
                for f in work:
                    f()
                return
            riders.extend([()] * skip)
            riders.extend(work[i * len(work) // n:(i + 1) * len(work) // n] for i in range(n))

        def up_ops(w_s, c):
            return _b_ops(*_quadrants(w_s, 0, KH, c_off[c], chunks[c] // 2))

        def up_proj(bops, lo=0, hi=TH):
            q = {}
            _strassen(lambda p: mm(get_xa(p, lo, hi), bops[p]()), q.__setitem__)
            return [q[i] for i in range(4)]

        def hidden(g, u):
            return _a_ops(*[_gelu_mul(a, b) for a, b in zip(g, u)])

        def down_ops(c):
            return _b_ops(*_quadrants(wd_s, c_off[c], chunks[c] // 2, 0, KH))

        def down(dops, ha, acc):
            out = {}
            for p in ORDER:
                v = mm(ha[p], dops[p]())
                out[p] = v if acc is None else acc[p] + v
            return out

        def project(t):
            def emit(i, quad):
                row0, j0 = (i // 2) * TH, (i % 2) * 4
                for j in range(4):
                    blk = quad[:, j * 128:(j + 1) * 128]
                    qkv_s[t, j0 + j, HALO + row0:HALO + row0 + TH, :] = blk
                    if row0 == 0 and t > 0:
                        qkv_s[t, j0 + j, 0:HALO, :] = jnp.broadcast_to(blk[0:1, :], (HALO, 128))
            w = jnp.concatenate([wp[t, r] for r in range(0, D, 16)], axis=0)
            bops = _b_ops(*_quadrants(w, 0, KH, 0, KH))
            _strassen(lambda p: mm(get_xa(p), bops[p]()), emit)

        def ffn_copies(lo, hi):
            return [cols(wg_hbm, wg_s, lo, hi), cols(wu_hbm, wu_s, lo, hi), rows(wd_hbm, wd_s, lo, hi)]

        def pin(*vals):
            wof_s[7, 0:8, :] = pltpu.bitcast(_zero_after(vals), F32)

        def finish_early(vals, pending):
            wait(pending)
            x_s[0:TH, 0:KH] = functools.reduce(jnp.add, vals).astype(BF)
            cp = copy(x_s, out_hbm)
            cp.start()
            cp.wait()

        cp_x = [[rows(x_hbm, x_s, t + b_off[b], t + b_off[b + 1]) for t in (0, TH)] for b in range(nb)]
        cp_g0, cp_u0, cp_d0 = ffn_copies(0, c_off[1])
        grp1 = ffn_copies(c_off[1], c_off[2]) + [copy(wqkv_hbm, wqkv_s)]
        grp2 = [copy(wo_hbm, wo_s)] + ffn_copies(c_off[2], DFU)
        cat = lambda parts: [jnp.concatenate(t, axis=0) for t in zip(*parts)]
        ln_work = lambda lo, hi: [functools.partial(ln_unit, r) for r in range(lo, hi, 16)]

        def take(quads, lo, hi):
            return [t[lo:hi] for t in quads]

        with scope("c0"):
            b1, b2, b3, b4 = b_off[1:5]
            b5 = b4 + RB
            start(cp_x[0] + [cp_g0, cp_u0] + sum(cp_x[1:], []) + [cp_d0] + grp1 + grp2)
            wait(cp_x[0])
            ride(ln_work(0, b1), 0)
            pin(*[a for r in range(0, b1, 16) for a in xa[r]])
            gops, uops = _once(up_ops(wg_s, 0)), _once(up_ops(wu_s, 0))
            dops = _once(down_ops(0))
            wait([cp_g0])
            g = [up_proj(gops, 0, b1)]
            wait([cp_u0] + cp_x[1])
            ride(ln_work(b1, b2), 0)
            u = [up_proj(uops, 0, b1)]
            if pin1:
                pin(*[a for r in range(b1, b2, 16) for a in xa[r]])
            wait(cp_x[2] + cp_x[3])
            ride(ln_work(b2, b4), 0)
            for lo, hi in ((b1, b2), (b2, b3)):
                g.append(up_proj(gops, lo, hi))
                u.append(up_proj(uops, lo, hi))
            if pin1:
                pin(*[a for r in range(b3, b4, 16) for a in xa[r]])
            wait(cp_x[4] + [cp_d0])
            ride(ln_work(b4, TH), 0)
            g, u, hs = cat(g), cat(u), {}

            def h_piece(r):
                hs[r] = hidden(take(g, r, r + 16), take(u, r, r + 16))
                return hs[r]
            ride([functools.partial(h_piece, r) for r in range(0, b3, 16)], h_n, 2)
            g2, u2 = [up_proj(gops, b3, b4)], [up_proj(uops, b3, b4)]
            acc0 = down(dops, cat([hs[r] for r in range(0, b3, 16)]), None)
            g2.append(up_proj(gops, b4, TH))
            u2.append(up_proj(uops, b4, TH))
            acc1 = down(dops, hidden(cat(g2), cat(u2)), None)
            acc = {p: jnp.concatenate([acc0[p], acc1[p]], axis=0) for p in ORDER}
        if stop == "c0":
            return finish_early(list(acc.values()), grp1 + grp2)

        with scope("c1"):
            wait(grp1)
            ride([functools.partial(permute_cols, t, r) for t in range(3) for r in range(0, D, 16)], perm_n, 2)
            acc = down(down_ops(1), hidden(up_proj(up_ops(wg_s, 1)), up_proj(up_ops(wu_s, 1))), acc)
            for t in range(3):
                project(t)
        if stop == "c1":
            return finish_early(list(acc.values()), grp2)

        with scope("ffn"):
            wait(grp2)
            for r in range(0, 16 * n_units, 16):
                attn_probs(r)
                attn_probs(TH + r)
            work = [functools.partial(permute_wo, j) for j in range(8)]
            work += [functools.partial(attn_mix, r, j) for r in range(0, 16 * n_units, 16) for j in range(4)]
            n_ride = (wo_at if wo_at is not None else len(chunks)) - pv_from
            for c in range(2, len(chunks)):
                n = c - pv_from
                if 0 <= n < n_ride:
                    ride(work[n * len(work) // n_ride:(n + 1) * len(work) // n_ride], pv_n)
                g = up_proj(up_ops(wg_s, c))
                if c == wo_at:
                    bops = _b_ops(*_quadrants(jnp.concatenate([wop[j] for j in range(8)], axis=1), 0, KH, 0, KH))
                    acc = {p: acc[p] + mm(get_oa(p), bops[p]()) for p in ORDER}
                ha = hidden(g, up_proj(up_ops(wu_s, c)))
                if c + 1 < len(chunks) or wo_at is None:
                    acc = down(down_ops(c), ha, acc)

            out_cps = []
            for j in range(KH // NO):
                lo, hi = slice(j * NO, (j + 1) * NO), slice(KH + j * NO, KH + (j + 1) * NO)
                if wo_at is None:
                    w_s, r0, k, lhs = jnp.concatenate([wop[i] for i in range(8)], axis=1), 0, KH, get_oa
                else:
                    w_s, r0, k, lhs = wd_s, c_off[-2], chunks[-1] // 2, lambda p: ha[p]
                bops = _b_ops(lambda: w_s[r0:r0 + k, lo], lambda: w_s[r0:r0 + k, hi],
                              lambda: w_s[r0 + k:r0 + 2 * k, lo], lambda: w_s[r0 + k:r0 + 2 * k, hi])

                def emit(i, quad):
                    rs, cs = slice((i // 2) * TH, (i // 2 + 1) * TH), (lo, hi)[i % 2]
                    x_s[rs, cs] = (x_s[rs, cs].astype(F32) + quad).astype(BF)
                    out_cps.append(copy(x_s.at[rs, cs], out_hbm.at[rs, cs]))
                    out_cps[-1].start()
                _strassen(lambda p: acc[p][:, lo] + mm(lhs(p), bops[p]()), emit)
            wait(out_cps)

    def fn(A_x, A_wqkv, A_wo, B_x, B_w_gate, B_w_up, B_w_down):
        del B_x
        hbm = pl.BlockSpec(memory_space=pl.ANY)
        out = pl.pallas_call(
            kernel,
            in_specs=[hbm] * 6,
            out_specs=hbm,
            out_shape=jax.ShapeDtypeStruct((S, D), BF),
            scratch_shapes=[
                pltpu.VMEM((S, D), BF),
                pltpu.VMEM((D, 3 * D), BF),
                pltpu.VMEM((3, 8, HALO + S, 128), F32),
                pltpu.VMEM((D, DF), BF),
                pltpu.VMEM((D, DF), BF),
                pltpu.VMEM((DF, D), BF),
                pltpu.VMEM((D, D), BF),
                pltpu.VMEM((8, H * STR, 128), F32),
                pltpu.SemaphoreType.DMA((2 * nb + 11 + 16,)),
            ],
            compiler_params=pltpu.CompilerParams(vmem_limit_bytes=vmem_mb * 1024 * 1024, flags=flags),
        )(A_x.reshape(S, D), A_wqkv, A_wo, B_w_gate, B_w_up, B_w_down)
        return out.reshape(1, S, D)
    return fn


_impl = make(**dict(flags={'XLA_TPU_EVENLY_DISTRIBUTE_CRITICAL_NODES': True}, h_n=0, pv_n=0, blocks=(192,128,128,128,448)))


@jax.jit
def pallas_parallel_sum__sliding_local_dilated__glu_gated_geglu__prompt_kernel(
    A_x: jax.Array,
    A_wqkv: jax.Array,
    A_wo: jax.Array,
    B_x: jax.Array,
    B_w_gate: jax.Array,
    B_w_up: jax.Array,
    B_w_down: jax.Array,
):
    return _impl(A_x, A_wqkv, A_wo, B_x, B_w_gate, B_w_up, B_w_down)
```

```python
import functools
import numpy as np
import jax
import jax.numpy as jnp
import jax.experimental.pallas as pl
import jax.experimental.pallas.tpu as pltpu

S, D, DF = 2048, 1024, 3584
H, DH, W, DIL = 32, 32, 8, 2
HALO = 16
TH = S // 2
KH = D // 2
BF, F32, U32 = jnp.bfloat16, jnp.float32, jnp.uint32
STR = 33
ORDER = (4, 2, 1, 3, 0, 6, 5)


def _dot(a, b):
    return jnp.dot(a, b, preferred_element_type=F32)


def _a_ops(a11, a12, a21, a22):
    return [t.astype(BF) for t in (a11 + a22, a21 + a22, a11, a22, a11 + a12, a21 - a11, a12 - a22)]


def _b_ops(b11, b12, b21, b22):
    f = lambda t: t.astype(F32)
    return [lambda: (f(b11()) + f(b22())).astype(BF),
            b11,
            lambda: (f(b12()) - f(b22())).astype(BF),
            lambda: (f(b21()) - f(b11())).astype(BF),
            b22,
            lambda: (f(b11()) + f(b12())).astype(BF),
            lambda: (f(b21()) + f(b22())).astype(BF)]


def _once(fs):
    vals = {}

    def get(i):
        if i not in vals:
            vals[i] = fs[i]()
        return vals[i]
    return [functools.partial(get, i) for i in range(len(fs))]


def _zero_after(vals):
    tiles = []
    for v in vals:
        v = pltpu.bitcast(v, U32)
        tiles += [v[r:r + 8, c:c + 128] for r in range(0, v.shape[0], 8) for c in range(0, v.shape[1], 128)]
    return (functools.reduce(jnp.bitwise_or, tiles) >> 31) >> 1


def _strassen(prod, emit):
    m5, m3 = prod(4), prod(2)
    emit(1, m3 + m5)
    m2, m4 = prod(1), prod(3)
    emit(2, m2 + m4)
    m1, m7 = prod(0), prod(6)
    emit(0, (m4 - m5) + m1 + m7)
    m6 = prod(5)
    emit(3, (m3 - m2) + m1 + m6)


def _quadrants(ref, r0, k, c0, n):
    return (lambda: ref[r0:r0 + k, c0:c0 + n], lambda: ref[r0:r0 + k, c0 + n:c0 + 2 * n],
            lambda: ref[r0 + k:r0 + 2 * k, c0:c0 + n], lambda: ref[r0 + k:r0 + 2 * k, c0 + n:c0 + 2 * n])


def _gelu_mul(g, u):
    c = float(np.sqrt(2.0 / np.pi))
    z = g * (c + (c * 0.044715) * (g * g))
    return ((0.5 * g) * u) * (1.0 + jnp.tanh(z))


def make(chunks=(512,) * 7, blocks=(192, 128, 128, 128, 448), RB=128, wo_at=None, NO=128, PR=64,
         n_units=64, flags=None, stop=None, vmem_mb=127, scopes=False, pv_n=0, ln_skip=2, ln_n=0, ln_n2=0, perm_n=40, pv_from=4, h_n=0, inplace=True, pin_h=3, split=False, mid=(320,), last=(576,)):
    DFU = sum(chunks)
    c_off = [sum(chunks[:i]) for i in range(len(chunks) + 1)]
    b_off = [sum(blocks[:i]) for i in range(len(blocks) + 1)]
    nb = len(blocks)

    def scope(name):
        import contextlib
        return jax.named_scope(name) if scopes else contextlib.nullcontext()

    def kernel(x_hbm, wqkv_hbm, wo_hbm, wg_hbm, wu_hbm, wd_hbm, out_hbm,
               x_s, wqkv_s, qkv_s, wg_s, wu_s, wd_s, wo_s, wof_s, sems):
        def copy(src, dst, group):
            return pltpu.make_async_copy(src, dst, sems.at[group])

        def cols(hbm, vmem, lo, hi, group):
            return copy(hbm.at[:, lo:hi], vmem.at[:, lo:hi], group)

        def rows(hbm, vmem, lo, hi, group):
            return copy(hbm.at[lo:hi, :], vmem.at[lo:hi, :], group)

        def start(cps):
            for cp in cps:
                cp.start()

        def wait(cps):
            for cp in cps:
                cp.wait()

        def ln(r, n):
            x = [x_s[r:r + n, j * 128:(j + 1) * 128].astype(F32) for j in range(D // 128)]
            lanesum = lambda t: jnp.broadcast_to(jnp.sum(t, axis=-1, keepdims=True), t.shape)
            mu = functools.reduce(jnp.add, x) * (128.0 / D)
            m2 = functools.reduce(jnp.add, [(t - mu) * (t - mu) for t in x])
            mean = lanesum(mu) * (1.0 / 128)
            dm = mu - mean
            var = lanesum(m2 + (D // 128) * (dm * dm)) * (1.0 / D)
            rs = jax.lax.rsqrt(var + 1e-5)
            return [(t - mean) * rs for t in x]

        xa = {}

        def ln_unit(r):
            top, bot = ln(r, 16), ln(TH + r, 16)
            ops = [_a_ops(top[j], top[j + 4], bot[j], bot[j + 4]) for j in range(4)]
            xa[r] = [jnp.concatenate(t, axis=1) for t in zip(*ops)]
            return xa[r]

        wp = {}

        def permute_cols(t, r):
            lane = jax.lax.broadcasted_iota(jnp.int32, (8, 128), 1)
            tiles = []
            for k in range(8):
                w = pltpu.bitcast(wqkv_s[r:r + 16, t * D + k * 128:t * D + (k + 1) * 128], U32)
                src = (lane - 4 * k) & 127
                idx = ((src & 3) << 5) | (src & 28) | (src >> 5)
                tiles.append(jnp.take_along_axis(w, idx, axis=1, mode="promise_in_bounds"))
            xs = [tiles[(-k) % 8] for k in range(8)]
            for b in range(3):
                sel = (lane & (4 << b)) != 0
                xs = [jnp.where(sel, xs[(k - (1 << b)) % 8], xs[k]) for k in range(8)]
            ys = [xs[j] if j == 0 else pltpu.roll(xs[j], 128 - 4 * j, 1) for j in range(8)]
            wp[t, r] = pltpu.bitcast(jnp.concatenate(ys, axis=1), BF)
            if inplace:
                wqkv_s[r:r + 16, t * D:(t + 1) * D] = wp[t, r]
            return [wp[t, r]]

        wop = {}

        def permute_wo(j):
            for h in range(H):
                wof_s[j, h * STR:h * STR + DH, :] = wo_s[h * DH:(h + 1) * DH, j * 128:(j + 1) * 128].astype(F32)
            wop[j] = jnp.concatenate([wof_s[j, pl.ds(d, H, stride=STR), :].astype(BF) for d in range(DH)], axis=0)
            return [wop[j]]

        c_exp = float(DH ** -0.5 * np.log2(np.e))
        neg = float(-1e9 / DH ** -0.5)

        def window(t, j, r, w):
            return qkv_s[t, j, HALO + r - DIL * w:HALO + r - DIL * w + 16, :]

        probs = {}

        def attn_probs(r):
            q = [window(0, j, r, 0) for j in range(8)]
            logits = []
            for w in range(W):
                pr = [q[j] * window(1, j, r, w) for j in range(8)]
                t = ((pr[0] + pr[1]) + (pr[2] + pr[3])) + ((pr[4] + pr[5]) + (pr[6] + pr[7]))
                t = t + pltpu.roll(t, 64, 1)
                t = t + pltpu.roll(t, 32, 1)
                if r < DIL * w:
                    pos = r + jax.lax.broadcasted_iota(jnp.int32, (16, 128), 0)
                    t = jnp.where(pos >= DIL * w, t, neg)
                logits.append(t)
            mx = functools.reduce(jnp.maximum, logits)
            e = [jnp.exp2((t - mx) * c_exp) for t in logits]
            inv = 1.0 / functools.reduce(jnp.add, e)
            probs[r] = [t * inv for t in e]
            return [inv]

        oa = {}

        def attn_mix(r, j):
            out = lambda r0, jj: functools.reduce(jnp.add, [probs[r0][w] * window(2, jj, r0, w) for w in range(W)])
            oa[r, j] = _a_ops(out(r, j), out(r, j + 4), out(TH + r, j), out(TH + r, j + 4))
            return oa[r, j]

        def get_xa(p, lo=0, hi=TH):
            return jnp.concatenate([xa[r][p] for r in range(lo, hi, 16)], axis=0)

        def get_oa(p):
            return jnp.concatenate([jnp.concatenate([oa[r % (16 * n_units), j][p] for j in range(4)], axis=1)
                                    for r in range(0, TH, 16)], axis=0)

        riders = []

        def paced(a, work):
            a = pltpu.bitcast(a, U32)
            step = a.shape[0] // 8 // len(work) * 8
            slabs = [a[:step // 16 * 8]] if step >= 16 else []
            for i, f in enumerate(work):
                lo = step // 16 * 8 + i * step
                slab = a[lo:lo + step if i + 1 < len(work) else a.shape[0]]
                head = jnp.concatenate([slab[0:8, 0:128] | _zero_after(f()), slab[0:8, 128:]], axis=1)
                slabs += [head, slab[8:]] if slab.shape[0] > 8 else [head]
            return pltpu.bitcast(jnp.concatenate(slabs, axis=0), BF)

        def mm(a, b):
            if not riders:
                return _dot(a, b)
            n = 128 * 512 // b.shape[0]
            outs = []
            for c in range(0, b.shape[1], n):
                work = riders.pop(0) if riders else ()
                outs.append(_dot(paced(a, work) if work else a, b[:, c:c + n]))
            return jnp.concatenate(outs, axis=1)

        def ride(work, n, skip=0):
            assert not riders
            if n == 0:
                for f in work:
                    f()
                return
            riders.extend([()] * skip)
            riders.extend(work[i * len(work) // n:(i + 1) * len(work) // n] for i in range(n))

        def up_ops(w_s, c):
            return _b_ops(*_quadrants(w_s, 0, KH, c_off[c], chunks[c] // 2))

        def up_proj(bops, lo=0, hi=TH):
            q = {}
            _strassen(lambda p: mm(get_xa(p, lo, hi), bops[p]()), q.__setitem__)
            return [q[i] for i in range(4)]

        def hidden(g, u):
            return _a_ops(*[_gelu_mul(a, b) for a, b in zip(g, u)])

        def down_ops(c):
            return _b_ops(*_quadrants(wd_s, c_off[c], chunks[c] // 2, 0, KH))

        def down(dops, ha, acc):
            out = {}
            for p in ORDER:
                v = mm(ha[p], dops[p]())
                out[p] = v if acc is None else acc[p] + v
            return out

        def project(t):
            def emit(i, quad):
                row0, j0 = (i // 2) * TH, (i % 2) * 4
                for j in range(4):
                    blk = quad[:, j * 128:(j + 1) * 128]
                    qkv_s[t, j0 + j, HALO + row0:HALO + row0 + TH, :] = blk
                    if row0 == 0 and t > 0:
                        qkv_s[t, j0 + j, 0:HALO, :] = jnp.broadcast_to(blk[0:1, :], (HALO, 128))
            w = jnp.concatenate([wp[t, r] for r in range(0, D, 16)], axis=0)
            bops = _b_ops(*(_quadrants(wqkv_s, 0, KH, t * D, KH) if inplace else _quadrants(w, 0, KH, 0, KH)))
            _strassen(lambda p: mm(get_xa(p), bops[p]()), emit)

        def ffn_copies(lo, hi, group):
            return [cols(wg_hbm, wg_s, lo, hi, group), cols(wu_hbm, wu_s, lo, hi, group),
                    rows(wd_hbm, wd_s, lo, hi, group)]

        def x_copies(lo, hi, group):
            return [rows(x_hbm, x_s, t + lo, t + hi, group) for t in (0, TH)]

        def pin(*vals):
            wof_s[7, 0:8, :] = pltpu.bitcast(_zero_after(vals), F32)

        def finish_early(vals, pending):
            wait(pending)
            x_s[0:TH, 0:KH] = functools.reduce(jnp.add, vals).astype(BF)
            cp = copy(x_s, out_hbm, 7)
            cp.start()
            cp.wait()

        b1, b2, b3, b4 = b_off[1:5]
        loads = [x_copies(0, b1, 0),
                 [cols(wg_hbm, wg_s, 0, c_off[1], 1)],
                 [cols(wu_hbm, wu_s, 0, c_off[1], 2)] + x_copies(b1, b2, 2),
                 x_copies(b2, b4, 3),
                 x_copies(b4, TH, 4) + [rows(wd_hbm, wd_s, 0, c_off[1], 4)],
                 ffn_copies(c_off[1], c_off[2], 5) + [copy(wqkv_hbm, wqkv_s, 5)],
                 [copy(wo_hbm, wo_s, 6)] + ffn_copies(c_off[2], DFU, 6)]
        grp1, grp2 = loads[5:]
        cat = lambda parts: [jnp.concatenate(t, axis=0) for t in zip(*parts)]
        ln_work = lambda lo, hi: [functools.partial(ln_unit, r) for r in range(lo, hi, 16)]

        def take(quads, lo, hi):
            return [t[lo:hi] for t in quads]

        def xa_vals(lo, hi):
            return [a for r in range(lo, hi, 16) for a in xa[r]]

        with scope("c0"):
            start(sum(loads, []))
            wait(loads[0])
            ride(ln_work(0, b1), 0)
            pin(*xa_vals(0, b1))
            gops, uops = _once(up_ops(wg_s, 0)), _once(up_ops(wu_s, 0))
            dops = _once(down_ops(0))
            block = lambda lo, hi: hidden(up_proj(gops, lo, hi), up_proj(uops, lo, hi))
            wait(loads[1])
            g = up_proj(gops, 0, b1)
            wait(loads[2])
            ride(ln_work(b1, b2), 0)
            hs = [hidden(g, up_proj(uops, 0, b1))]
            pin(*(xa_vals(b1, b2) + (hs[0] if pin_h & 1 else [])))
            wait(loads[3])
            ride(ln_work(b2, b4), 0)
            hs += [block(lo, hi) for lo, hi in zip((b1,) + mid, mid + (b3,))]
            pin(*(xa_vals(b3, b4) + (sum(hs[1:], []) if pin_h & 2 else [])))
            wait(loads[4])
            ride(ln_work(b4, TH), 0)
            tail = list(zip((b3,) + last, last + (TH,)))
            if split:
                hs2 = [block(*tail[0])]
                acc0 = down(dops, cat(hs), None)
                hs2 += [block(*t) for t in tail[1:]]
                acc1 = down(dops, cat(hs2), None)
                acc = {p: jnp.concatenate([acc0[p], acc1[p]], axis=0) for p in ORDER}
            else:
                acc = down(dops, cat(hs + [block(*t) for t in tail]), None)
        if stop == "c0":
            return finish_early(list(acc.values()), grp1 + grp2)

        with scope("c1"):
            wait(grp1)
            ride([functools.partial(permute_cols, t, r) for t in range(3) for r in range(0, D, 16)], perm_n, 2)
            acc = down(down_ops(1), hidden(up_proj(up_ops(wg_s, 1)), up_proj(up_ops(wu_s, 1))), acc)
            for t in range(3):
                project(t)
        if stop == "c1":
            return finish_early(list(acc.values()), grp2)

        with scope("ffn"):
            wait(grp2)
            for r in range(0, 16 * n_units, 16):
                attn_probs(r)
                attn_probs(TH + r)
            work = [functools.partial(permute_wo, j) for j in range(8)]
            work += [functools.partial(attn_mix, r, j) for r in range(0, 16 * n_units, 16) for j in range(4)]
            n_ride = (wo_at if wo_at is not None else len(chunks)) - pv_from
            for c in range(2, len(chunks)):
                n = c - pv_from
                if 0 <= n < n_ride:
                    ride(work[n * len(work) // n_ride:(n + 1) * len(work) // n_ride], pv_n)
                g = up_proj(up_ops(wg_s, c))
                if c == wo_at:
                    bops = _b_ops(*_quadrants(jnp.concatenate([wop[j] for j in range(8)], axis=1), 0, KH, 0, KH))
                    acc = {p: acc[p] + mm(get_oa(p), bops[p]()) for p in ORDER}
                ha = hidden(g, up_proj(up_ops(wu_s, c)))
                if c + 1 < len(chunks) or wo_at is None:
                    acc = down(down_ops(c), ha, acc)

            out_cps = []
            for j in range(KH // NO):
                lo, hi = slice(j * NO, (j + 1) * NO), slice(KH + j * NO, KH + (j + 1) * NO)
                if wo_at is None:
                    w_s, r0, k, lhs = jnp.concatenate([wop[i] for i in range(8)], axis=1), 0, KH, get_oa
                else:
                    w_s, r0, k, lhs = wd_s, c_off[-2], chunks[-1] // 2, lambda p: ha[p]
                bops = _b_ops(lambda: w_s[r0:r0 + k, lo], lambda: w_s[r0:r0 + k, hi],
                              lambda: w_s[r0 + k:r0 + 2 * k, lo], lambda: w_s[r0 + k:r0 + 2 * k, hi])

                def emit(i, quad):
                    rs, cs = slice((i // 2) * TH, (i // 2 + 1) * TH), (lo, hi)[i % 2]
                    x_s[rs, cs] = (x_s[rs, cs].astype(F32) + quad).astype(BF)
                    out_cps.append(copy(x_s.at[rs, cs], out_hbm.at[rs, cs], 7))
                    out_cps[-1].start()
                _strassen(lambda p: acc[p][:, lo] + mm(lhs(p), bops[p]()), emit)
            wait(out_cps)

    def fn(A_x, A_wqkv, A_wo, B_x, B_w_gate, B_w_up, B_w_down):
        del B_x
        hbm = pl.BlockSpec(memory_space=pl.ANY)
        out = pl.pallas_call(
            kernel,
            in_specs=[hbm] * 6,
            out_specs=hbm,
            out_shape=jax.ShapeDtypeStruct((S, D), BF),
            scratch_shapes=[
                pltpu.VMEM((S, D), BF),
                pltpu.VMEM((D, 3 * D), BF),
                pltpu.VMEM((3, 8, HALO + S, 128), F32),
                pltpu.VMEM((D, DF), BF),
                pltpu.VMEM((D, DF), BF),
                pltpu.VMEM((DF, D), BF),
                pltpu.VMEM((D, D), BF),
                pltpu.VMEM((8, H * STR, 128), F32),
                pltpu.SemaphoreType.DMA((8,)),
            ],
            compiler_params=pltpu.CompilerParams(vmem_limit_bytes=vmem_mb * 1024 * 1024, flags=flags),
        )(A_x.reshape(S, D), A_wqkv, A_wo, B_w_gate, B_w_up, B_w_down)
        return out.reshape(1, S, D)
    return fn


_impl = make(**dict(flags={'XLA_TPU_EVENLY_DISTRIBUTE_CRITICAL_NODES': True}, pin_h=0,split=True,blocks=(192,96,160,128,448),mid=(288,),last=(576,704)))


@jax.jit
def pallas_parallel_sum__sliding_local_dilated__glu_gated_geglu__prompt_kernel(
    A_x: jax.Array,
    A_wqkv: jax.Array,
    A_wo: jax.Array,
    B_x: jax.Array,
    B_w_gate: jax.Array,
    B_w_up: jax.Array,
    B_w_down: jax.Array,
):
    return _impl(A_x, A_wqkv, A_wo, B_x, B_w_gate, B_w_up, B_w_down)
```

```python
import functools
import numpy as np
import jax
import jax.numpy as jnp
import jax.experimental.pallas as pl
import jax.experimental.pallas.tpu as pltpu

S, D, DF = 2048, 1024, 3584
H, DH, W, DIL = 32, 32, 8, 2
HALO = 16
TH = S // 2
KH = D // 2
BF, F32, U32 = jnp.bfloat16, jnp.float32, jnp.uint32
STR = 33
ORDER = (4, 2, 1, 3, 0, 6, 5)


def _dot(a, b):
    return jnp.dot(a, b, preferred_element_type=F32)


def _a_ops(a11, a12, a21, a22):
    return [t.astype(BF) for t in (a11 + a22, a21 + a22, a11, a22, a11 + a12, a21 - a11, a12 - a22)]


def _b_ops(b11, b12, b21, b22):
    f = lambda t: t.astype(F32)
    return [lambda: (f(b11()) + f(b22())).astype(BF),
            b11,
            lambda: (f(b12()) - f(b22())).astype(BF),
            lambda: (f(b21()) - f(b11())).astype(BF),
            b22,
            lambda: (f(b11()) + f(b12())).astype(BF),
            lambda: (f(b21()) + f(b22())).astype(BF)]


def _once(fs):
    vals = {}

    def get(i):
        if i not in vals:
            vals[i] = fs[i]()
        return vals[i]
    return [functools.partial(get, i) for i in range(len(fs))]


def _zero_after(vals):
    tiles = []
    for v in vals:
        v = pltpu.bitcast(v, U32)
        tiles += [v[r:r + 8, c:c + 128] for r in range(0, v.shape[0], 8) for c in range(0, v.shape[1], 128)]
    return (functools.reduce(jnp.bitwise_or, tiles) >> 31) >> 1


def _strassen(prod, emit):
    m5, m3 = prod(4), prod(2)
    emit(1, m3 + m5)
    m2, m4 = prod(1), prod(3)
    emit(2, m2 + m4)
    m1, m7 = prod(0), prod(6)
    emit(0, (m4 - m5) + m1 + m7)
    m6 = prod(5)
    emit(3, (m3 - m2) + m1 + m6)


def _quadrants(ref, r0, k, c0, n):
    return (lambda: ref[r0:r0 + k, c0:c0 + n], lambda: ref[r0:r0 + k, c0 + n:c0 + 2 * n],
            lambda: ref[r0 + k:r0 + 2 * k, c0:c0 + n], lambda: ref[r0 + k:r0 + 2 * k, c0 + n:c0 + 2 * n])


def _gelu_mul(g, u):
    c = float(np.sqrt(2.0 / np.pi))
    z = g * (c + (c * 0.044715) * (g * g))
    return ((0.5 * g) * u) * (1.0 + jnp.tanh(z))


def make(chunks=(512,) * 7, blocks=(192, 96, 160, 128, 448), RB=128, wo_at=None, NO=128, PR=64,
         n_units=64, flags=None, stop=None, vmem_mb=127, scopes=False, pv_n=0, ln_skip=2, ln_n=0, ln_n2=0, perm_n=40, pv_from=4, h_n=0, inplace=True, pin_h=0, split=True, mid=(288,), last=(576, 704), prio=0, halves=False, lag=16, full_p=False):
    DFU = sum(chunks)
    c_off = [sum(chunks[:i]) for i in range(len(chunks) + 1)]
    b_off = [sum(blocks[:i]) for i in range(len(blocks) + 1)]
    nb = len(blocks)

    def scope(name):
        import contextlib
        return jax.named_scope(name) if scopes else contextlib.nullcontext()

    def kernel(x_hbm, wqkv_hbm, wo_hbm, wg_hbm, wu_hbm, wd_hbm, out_hbm,
               x_s, wqkv_s, qkv_s, wg_s, wu_s, wd_s, wo_s, wof_s, sems):
        def copy(src, dst, group):
            return pltpu.make_async_copy(src, dst, sems.at[group])

        def cols(hbm, vmem, lo, hi, group):
            return copy(hbm.at[:, lo:hi], vmem.at[:, lo:hi], group)

        def rows(hbm, vmem, lo, hi, group):
            return copy(hbm.at[lo:hi, :], vmem.at[lo:hi, :], group)

        def start(cps):
            for i, cp in enumerate(cps):
                cp.start(priority=i % 2 if prio == 2 else prio)

        wait_id = iter(range(100))

        def wait(cps):
            with scope(f"wait{next(wait_id)}"):
                for cp in cps:
                    cp.wait()

        def ln(r, n):
            x = [x_s[r:r + n, j * 128:(j + 1) * 128].astype(F32) for j in range(D // 128)]
            lanesum = lambda t: jnp.broadcast_to(jnp.sum(t, axis=-1, keepdims=True), t.shape)
            mu = functools.reduce(jnp.add, x) * (128.0 / D)
            m2 = functools.reduce(jnp.add, [(t - mu) * (t - mu) for t in x])
            mean = lanesum(mu) * (1.0 / 128)
            dm = mu - mean
            var = lanesum(m2 + (D // 128) * (dm * dm)) * (1.0 / D)
            rs = jax.lax.rsqrt(var + 1e-5)
            return [(t - mean) * rs for t in x]

        xa = {}

        def ln_unit(r):
            top, bot = ln(r, 16), ln(TH + r, 16)
            ops = [_a_ops(top[j], top[j + 4], bot[j], bot[j + 4]) for j in range(4)]
            xa[r] = [jnp.concatenate(t, axis=1) for t in zip(*ops)]
            return xa[r]

        wp = {}

        def permute_cols(t, r):
            lane = jax.lax.broadcasted_iota(jnp.int32, (8, 128), 1)
            tiles = []
            for k in range(8):
                w = pltpu.bitcast(wqkv_s[r:r + 16, t * D + k * 128:t * D + (k + 1) * 128], U32)
                src = (lane - 4 * k) & 127
                idx = ((src & 3) << 5) | (src & 28) | (src >> 5)
                tiles.append(jnp.take_along_axis(w, idx, axis=1, mode="promise_in_bounds"))
            xs = [tiles[(-k) % 8] for k in range(8)]
            for b in range(3):
                sel = (lane & (4 << b)) != 0
                xs = [jnp.where(sel, xs[(k - (1 << b)) % 8], xs[k]) for k in range(8)]
            ys = [xs[j] if j == 0 else pltpu.roll(xs[j], 128 - 4 * j, 1) for j in range(8)]
            wp[t, r] = pltpu.bitcast(jnp.concatenate(ys, axis=1), BF)
            if inplace:
                wqkv_s[r:r + 16, t * D:(t + 1) * D] = wp[t, r]
            return [wp[t, r]]

        wop = {}

        def permute_wo(j):
            for h in range(H):
                wof_s[j, h * STR:h * STR + DH, :] = wo_s[h * DH:(h + 1) * DH, j * 128:(j + 1) * 128].astype(F32)
            wop[j] = jnp.concatenate([wof_s[j, pl.ds(d, H, stride=STR), :].astype(BF) for d in range(DH)], axis=0)
            return [wop[j]]

        c_exp = float(DH ** -0.5 * np.log2(np.e))
        neg = float(-1e9 / DH ** -0.5)

        def window(t, j, r, w):
            return qkv_s[t, j, HALO + r - DIL * w:HALO + r - DIL * w + 16, :]

        probs = {}

        def attn_probs(r, dep=None):
            q = [window(0, j, r, 0) for j in range(8)]
            logits = []
            for w in range(W):
                pr = [q[j] * window(1, j, r, w) for j in range(8)]
                t = ((pr[0] + pr[1]) + (pr[2] + pr[3])) + ((pr[4] + pr[5]) + (pr[6] + pr[7]))
                if dep is not None and w == 0:
                    t = jnp.concatenate([pltpu.bitcast(pltpu.bitcast(t[0:8], U32) | dep, F32), t[8:]], axis=0)
                t = t + pltpu.roll(t, 64, 1)
                t = t + pltpu.roll(t, 32, 1)
                if r < DIL * w:
                    pos = r + jax.lax.broadcasted_iota(jnp.int32, (16, 128), 0)
                    t = jnp.where(pos >= DIL * w, t, neg)
                logits.append(t)
            mx = functools.reduce(jnp.maximum, logits)
            e = [jnp.exp2((t - mx) * c_exp) for t in logits]
            inv = 1.0 / functools.reduce(jnp.add, e)
            probs[r] = [t * inv for t in e]
            return probs[r] if full_p else [inv]

        oa = {}

        def attn_mix(r, j):
            out = lambda r0, jj: functools.reduce(jnp.add, [probs[r0][w] * window(2, jj, r0, w) for w in range(W)])
            oa[r, j] = _a_ops(out(r, j), out(r, j + 4), out(TH + r, j), out(TH + r, j + 4))
            return oa[r, j]

        def get_xa(p, lo=0, hi=TH):
            return jnp.concatenate([xa[r][p] for r in range(lo, hi, 16)], axis=0)

        def get_oa(p):
            return jnp.concatenate([jnp.concatenate([oa[r % (16 * n_units), j][p] for j in range(4)], axis=1)
                                    for r in range(0, TH, 16)], axis=0)

        riders = []

        def paced(a, work):
            a = pltpu.bitcast(a, U32)
            step = a.shape[0] // 8 // len(work) * 8
            slabs = [a[:step // 16 * 8]] if step >= 16 else []
            for i, f in enumerate(work):
                lo = step // 16 * 8 + i * step
                slab = a[lo:lo + step if i + 1 < len(work) else a.shape[0]]
                head = jnp.concatenate([slab[0:8, 0:128] | _zero_after(f()), slab[0:8, 128:]], axis=1)
                slabs += [head, slab[8:]] if slab.shape[0] > 8 else [head]
            return pltpu.bitcast(jnp.concatenate(slabs, axis=0), BF)

        def mm(a, b):
            if not riders:
                return _dot(a, b)
            n = 128 * 512 // b.shape[0]
            outs = []
            for c in range(0, b.shape[1], n):
                work = riders.pop(0) if riders else ()
                outs.append(_dot(paced(a, work) if work else a, b[:, c:c + n]))
            return jnp.concatenate(outs, axis=1)

        def ride(work, n, skip=0):
            assert not riders
            if n == 0:
                for f in work:
                    f()
                return
            riders.extend([()] * skip)
            riders.extend(work[i * len(work) // n:(i + 1) * len(work) // n] for i in range(n))

        def up_ops(w_s, c):
            return _b_ops(*_quadrants(w_s, 0, KH, c_off[c], chunks[c] // 2))

        def up_proj(bops, lo=0, hi=TH):
            q = {}
            _strassen(lambda p: mm(get_xa(p, lo, hi), bops[p]()), q.__setitem__)
            return [q[i] for i in range(4)]

        def hidden(g, u):
            return _a_ops(*[_gelu_mul(a, b) for a, b in zip(g, u)])

        def down_ops(c):
            return _b_ops(*_quadrants(wd_s, c_off[c], chunks[c] // 2, 0, KH))

        def down(dops, ha, acc):
            out = {}
            for p in ORDER:
                v = mm(ha[p], dops[p]())
                out[p] = v if acc is None else acc[p] + v
            return out

        def project(t):
            def emit(i, quad):
                row0, j0 = (i // 2) * TH, (i % 2) * 4
                for j in range(4):
                    blk = quad[:, j * 128:(j + 1) * 128]
                    qkv_s[t, j0 + j, HALO + row0:HALO + row0 + TH, :] = blk
                    if row0 == 0 and t > 0:
                        qkv_s[t, j0 + j, 0:HALO, :] = jnp.broadcast_to(blk[0:1, :], (HALO, 128))
            w = jnp.concatenate([wp[t, r] for r in range(0, D, 16)], axis=0)
            bops = _b_ops(*(_quadrants(wqkv_s, 0, KH, t * D, KH) if inplace else _quadrants(w, 0, KH, 0, KH)))
            _strassen(lambda p: mm(get_xa(p), bops[p]()), emit)

        def ffn_copies(lo, hi, group):
            return [cols(wg_hbm, wg_s, lo, hi, group), cols(wu_hbm, wu_s, lo, hi, group),
                    rows(wd_hbm, wd_s, lo, hi, group)]

        def x_copies(lo, hi, group):
            return [rows(x_hbm, x_s, t + lo, t + hi, group) for t in (0, TH)]

        def pin(*vals):
            wof_s[7, 0:8, :] = pltpu.bitcast(_zero_after(vals), F32)

        def finish_early(vals, pending):
            wait(pending)
            x_s[0:TH, 0:KH] = functools.reduce(jnp.add, vals).astype(BF)
            cp = copy(x_s, out_hbm, 7)
            cp.start()
            cp.wait()

        b1, b2, b3, b4 = b_off[1:5]

        def first(hbm, vmem, group):
            if not halves:
                return [cols(hbm, vmem, 0, c_off[1], group)]
            return [copy(hbm.at[r:r + KH, 0:c_off[1]], vmem.at[r:r + KH, 0:c_off[1]], group) for r in (0, KH)]
        loads = [x_copies(0, b1, 0),
                 first(wg_hbm, wg_s, 1),
                 first(wu_hbm, wu_s, 2) + x_copies(b1, b2, 2),
                 x_copies(b2, b4, 3),
                 x_copies(b4, TH, 4) + [rows(wd_hbm, wd_s, 0, c_off[1], 4)],
                 ffn_copies(c_off[1], c_off[2], 5) + [copy(wqkv_hbm, wqkv_s, 5)],
                 [copy(wo_hbm, wo_s, 6)] + ffn_copies(c_off[2], DFU, 6)]
        grp1, grp2 = loads[5:]
        cat = lambda parts: [jnp.concatenate(t, axis=0) for t in zip(*parts)]
        ln_work = lambda lo, hi: [functools.partial(ln_unit, r) for r in range(lo, hi, 16)]

        def take(quads, lo, hi):
            return [t[lo:hi] for t in quads]

        def xa_vals(lo, hi):
            return [a for r in range(lo, hi, 16) for a in xa[r]]

        with scope("c0"):
            start(sum(loads, []))
            wait(loads[0])
            ride(ln_work(0, b1), 0)
            pin(*xa_vals(0, b1))
            gops, uops = _once(up_ops(wg_s, 0)), _once(up_ops(wu_s, 0))
            dops = _once(down_ops(0))
            block = lambda lo, hi: hidden(up_proj(gops, lo, hi), up_proj(uops, lo, hi))
            wait(loads[1])
            g = up_proj(gops, 0, b1)
            wait(loads[2])
            ride(ln_work(b1, b2), 0)
            hs = [hidden(g, up_proj(uops, 0, b1))]
            pin(*(xa_vals(b1, b2) + (hs[0] if pin_h & 1 else [])))
            wait(loads[3])
            ride(ln_work(b2, b4), 0)
            hs += [block(lo, hi) for lo, hi in zip((b1,) + mid, mid + (b3,))]
            pin(*(xa_vals(b3, b4) + (sum(hs[1:], []) if pin_h & 2 else [])))
            wait(loads[4])
            ride(ln_work(b4, TH), 0)
            tail = list(zip((b3,) + last, last + (TH,)))
            if split:
                hs2 = [block(*tail[0])]
                acc0 = down(dops, cat(hs), None)
                hs2 += [block(*t) for t in tail[1:]]
                acc1 = down(dops, cat(hs2), None)
                acc = {p: jnp.concatenate([acc0[p], acc1[p]], axis=0) for p in ORDER}
            else:
                acc = down(dops, cat(hs + [block(*t) for t in tail]), None)
        if stop == "c0":
            return finish_early(list(acc.values()), grp1 + grp2)

        with scope("c1"):
            wait(grp1)
            ride([functools.partial(permute_cols, t, r) for t in range(3) for r in range(0, D, 16)], perm_n, 2)
            acc = down(down_ops(1), hidden(up_proj(up_ops(wg_s, 1)), up_proj(up_ops(wu_s, 1))), acc)
            for t in range(3):
                project(t)
        if stop == "c1":
            return finish_early(list(acc.values()), grp2)

        with scope("ffn"):
            wait(grp2)
            done = []
            for r in range(0, 16 * n_units, 16):
                for t in (0, TH):
                    dep = _zero_after(done[-lag]) if lag and len(done) >= lag else None
                    done.append(attn_probs(t + r, dep))
            work = [functools.partial(permute_wo, j) for j in range(8)]
            work += [functools.partial(attn_mix, r, j) for r in range(0, 16 * n_units, 16) for j in range(4)]
            n_ride = (wo_at if wo_at is not None else len(chunks)) - pv_from
            for c in range(2, len(chunks)):
                n = c - pv_from
                if 0 <= n < n_ride:
                    ride(work[n * len(work) // n_ride:(n + 1) * len(work) // n_ride], pv_n)
                g = up_proj(up_ops(wg_s, c))
                if c == wo_at:
                    bops = _b_ops(*_quadrants(jnp.concatenate([wop[j] for j in range(8)], axis=1), 0, KH, 0, KH))
                    acc = {p: acc[p] + mm(get_oa(p), bops[p]()) for p in ORDER}
                ha = hidden(g, up_proj(up_ops(wu_s, c)))
                if c + 1 < len(chunks) or wo_at is None:
                    acc = down(down_ops(c), ha, acc)

            out_cps = []
            for j in range(KH // NO):
                lo, hi = slice(j * NO, (j + 1) * NO), slice(KH + j * NO, KH + (j + 1) * NO)
                if wo_at is None:
                    w_s, r0, k, lhs = jnp.concatenate([wop[i] for i in range(8)], axis=1), 0, KH, get_oa
                else:
                    w_s, r0, k, lhs = wd_s, c_off[-2], chunks[-1] // 2, lambda p: ha[p]
                bops = _b_ops(lambda: w_s[r0:r0 + k, lo], lambda: w_s[r0:r0 + k, hi],
                              lambda: w_s[r0 + k:r0 + 2 * k, lo], lambda: w_s[r0 + k:r0 + 2 * k, hi])

                def emit(i, quad):
                    rs, cs = slice((i // 2) * TH, (i // 2 + 1) * TH), (lo, hi)[i % 2]
                    x_s[rs, cs] = (x_s[rs, cs].astype(F32) + quad).astype(BF)
                    out_cps.append(copy(x_s.at[rs, cs], out_hbm.at[rs, cs], 7))
                    out_cps[-1].start()
                _strassen(lambda p: acc[p][:, lo] + mm(lhs(p), bops[p]()), emit)
            wait(out_cps)

    def fn(A_x, A_wqkv, A_wo, B_x, B_w_gate, B_w_up, B_w_down):
        del B_x
        hbm = pl.BlockSpec(memory_space=pl.ANY)
        out = pl.pallas_call(
            kernel,
            in_specs=[hbm] * 6,
            out_specs=hbm,
            out_shape=jax.ShapeDtypeStruct((S, D), BF),
            scratch_shapes=[
                pltpu.VMEM((S, D), BF),
                pltpu.VMEM((D, 3 * D), BF),
                pltpu.VMEM((3, 8, HALO + S, 128), F32),
                pltpu.VMEM((D, DF), BF),
                pltpu.VMEM((D, DF), BF),
                pltpu.VMEM((DF, D), BF),
                pltpu.VMEM((D, D), BF),
                pltpu.VMEM((8, H * STR, 128), F32),
                pltpu.SemaphoreType.DMA((8,)),
            ],
            compiler_params=pltpu.CompilerParams(vmem_limit_bytes=vmem_mb * 1024 * 1024, flags=flags),
        )(A_x.reshape(S, D), A_wqkv, A_wo, B_w_gate, B_w_up, B_w_down)
        return out.reshape(1, S, D)
    return fn


_impl = make(**dict(flags={'XLA_TPU_EVENLY_DISTRIBUTE_CRITICAL_NODES': True}, lag=8, full_p=True))


@jax.jit
def pallas_parallel_sum__sliding_local_dilated__glu_gated_geglu__prompt_kernel(
    A_x: jax.Array,
    A_wqkv: jax.Array,
    A_wo: jax.Array,
    B_x: jax.Array,
    B_w_gate: jax.Array,
    B_w_up: jax.Array,
    B_w_down: jax.Array,
):
    return _impl(A_x, A_wqkv, A_wo, B_x, B_w_gate, B_w_up, B_w_down)
```

```python
import functools
import numpy as np
import jax
import jax.numpy as jnp
import jax.experimental.pallas as pl
import jax.experimental.pallas.tpu as pltpu

S, D, DF = 2048, 1024, 3584
H, DH, W, DIL = 32, 32, 8, 2
HALO = 16
TH = S // 2
KH = D // 2
BF, F32, U32 = jnp.bfloat16, jnp.float32, jnp.uint32
STR = 33
ORDER = (4, 2, 1, 3, 0, 6, 5)


def _dot(a, b):
    return jnp.dot(a, b, preferred_element_type=F32)


def _a_ops(a11, a12, a21, a22):
    return [t.astype(BF) for t in (a11 + a22, a21 + a22, a11, a22, a11 + a12, a21 - a11, a12 - a22)]


def _b_ops(b11, b12, b21, b22):
    f = lambda t: t.astype(F32)
    return [lambda: (f(b11()) + f(b22())).astype(BF),
            b11,
            lambda: (f(b12()) - f(b22())).astype(BF),
            lambda: (f(b21()) - f(b11())).astype(BF),
            b22,
            lambda: (f(b11()) + f(b12())).astype(BF),
            lambda: (f(b21()) + f(b22())).astype(BF)]


def _once(fs):
    vals = {}

    def get(i):
        if i not in vals:
            vals[i] = fs[i]()
        return vals[i]
    return [functools.partial(get, i) for i in range(len(fs))]


def _zero_after(vals):
    tiles = []
    for v in vals:
        v = pltpu.bitcast(v, U32)
        tiles += [v[r:r + 8, c:c + 128] for r in range(0, v.shape[0], 8) for c in range(0, v.shape[1], 128)]
    return (functools.reduce(jnp.bitwise_or, tiles) >> 31) >> 1


def _strassen(prod, emit):
    m5, m3 = prod(4), prod(2)
    emit(1, m3 + m5)
    m2, m4 = prod(1), prod(3)
    emit(2, m2 + m4)
    m1, m7 = prod(0), prod(6)
    emit(0, (m4 - m5) + m1 + m7)
    m6 = prod(5)
    emit(3, (m3 - m2) + m1 + m6)


def _quadrants(ref, r0, k, c0, n):
    return (lambda: ref[r0:r0 + k, c0:c0 + n], lambda: ref[r0:r0 + k, c0 + n:c0 + 2 * n],
            lambda: ref[r0 + k:r0 + 2 * k, c0:c0 + n], lambda: ref[r0 + k:r0 + 2 * k, c0 + n:c0 + 2 * n])


def _gelu_mul(g, u):
    c = float(np.sqrt(2.0 / np.pi))
    z = g * (c + (c * 0.044715) * (g * g))
    return ((0.5 * g) * u) * (1.0 + jnp.tanh(z))


def make(chunks=(512,) * 7, blocks=(192, 64, 192, 128, 448), RB=128, wo_at=None, NO=128, PR=64,
         n_units=64, flags=None, stop=None, vmem_mb=127, scopes=False, pv_n=0, ln_skip=2, ln_n=0, ln_n2=0, perm_n=40, pv_from=4, h_n=0, inplace=True, pin_h=0, split=True, mid=(256,), last=(576, 704), prio=0, halves=False, lag=8, full_p=True, early=3, x0a=96):
    DFU = sum(chunks)
    c_off = [sum(chunks[:i]) for i in range(len(chunks) + 1)]
    b_off = [sum(blocks[:i]) for i in range(len(blocks) + 1)]
    nb = len(blocks)

    def scope(name):
        import contextlib
        return jax.named_scope(name) if scopes else contextlib.nullcontext()

    def kernel(x_hbm, wqkv_hbm, wo_hbm, wg_hbm, wu_hbm, wd_hbm, out_hbm,
               x_s, wqkv_s, qkv_s, wg_s, wu_s, wd_s, wo_s, wof_s, sems):
        def copy(src, dst, group):
            return pltpu.make_async_copy(src, dst, sems.at[group])

        def cols(hbm, vmem, lo, hi, group):
            return copy(hbm.at[:, lo:hi], vmem.at[:, lo:hi], group)

        def rows(hbm, vmem, lo, hi, group):
            return copy(hbm.at[lo:hi, :], vmem.at[lo:hi, :], group)

        def start(cps):
            for i, cp in enumerate(cps):
                cp.start(priority=i % 2 if prio == 2 else prio)

        wait_id = iter(range(100))

        def wait(cps):
            with scope(f"wait{next(wait_id)}"):
                for cp in cps:
                    cp.wait()

        def ln(r, n):
            x = [x_s[r:r + n, j * 128:(j + 1) * 128].astype(F32) for j in range(D // 128)]
            lanesum = lambda t: jnp.broadcast_to(jnp.sum(t, axis=-1, keepdims=True), t.shape)
            mu = functools.reduce(jnp.add, x) * (128.0 / D)
            m2 = functools.reduce(jnp.add, [(t - mu) * (t - mu) for t in x])
            mean = lanesum(mu) * (1.0 / 128)
            dm = mu - mean
            var = lanesum(m2 + (D // 128) * (dm * dm)) * (1.0 / D)
            rs = jax.lax.rsqrt(var + 1e-5)
            return [(t - mean) * rs for t in x]

        xa = {}

        def ln_unit(r):
            top, bot = ln(r, 16), ln(TH + r, 16)
            ops = [_a_ops(top[j], top[j + 4], bot[j], bot[j + 4]) for j in range(4)]
            xa[r] = [jnp.concatenate(t, axis=1) for t in zip(*ops)]
            return xa[r]

        wp = {}

        def permute_cols(t, r):
            lane = jax.lax.broadcasted_iota(jnp.int32, (8, 128), 1)
            tiles = []
            for k in range(8):
                w = pltpu.bitcast(wqkv_s[r:r + 16, t * D + k * 128:t * D + (k + 1) * 128], U32)
                src = (lane - 4 * k) & 127
                idx = ((src & 3) << 5) | (src & 28) | (src >> 5)
                tiles.append(jnp.take_along_axis(w, idx, axis=1, mode="promise_in_bounds"))
            xs = [tiles[(-k) % 8] for k in range(8)]
            for b in range(3):
                sel = (lane & (4 << b)) != 0
                xs = [jnp.where(sel, xs[(k - (1 << b)) % 8], xs[k]) for k in range(8)]
            ys = [xs[j] if j == 0 else pltpu.roll(xs[j], 128 - 4 * j, 1) for j in range(8)]
            wp[t, r] = pltpu.bitcast(jnp.concatenate(ys, axis=1), BF)
            if inplace:
                wqkv_s[r:r + 16, t * D:(t + 1) * D] = wp[t, r]
            return [wp[t, r]]

        wop = {}

        def permute_wo(j):
            for h in range(H):
                wof_s[j, h * STR:h * STR + DH, :] = wo_s[h * DH:(h + 1) * DH, j * 128:(j + 1) * 128].astype(F32)
            wop[j] = jnp.concatenate([wof_s[j, pl.ds(d, H, stride=STR), :].astype(BF) for d in range(DH)], axis=0)
            return [wop[j]]

        c_exp = float(DH ** -0.5 * np.log2(np.e))
        neg = float(-1e9 / DH ** -0.5)

        def window(t, j, r, w):
            return qkv_s[t, j, HALO + r - DIL * w:HALO + r - DIL * w + 16, :]

        probs = {}

        def attn_probs(r, dep=None):
            q = [window(0, j, r, 0) for j in range(8)]
            logits = []
            for w in range(W):
                pr = [q[j] * window(1, j, r, w) for j in range(8)]
                t = ((pr[0] + pr[1]) + (pr[2] + pr[3])) + ((pr[4] + pr[5]) + (pr[6] + pr[7]))
                if dep is not None and w == 0:
                    t = jnp.concatenate([pltpu.bitcast(pltpu.bitcast(t[0:8], U32) | dep, F32), t[8:]], axis=0)
                t = t + pltpu.roll(t, 64, 1)
                t = t + pltpu.roll(t, 32, 1)
                if r < DIL * w:
                    pos = r + jax.lax.broadcasted_iota(jnp.int32, (16, 128), 0)
                    t = jnp.where(pos >= DIL * w, t, neg)
                logits.append(t)
            mx = functools.reduce(jnp.maximum, logits)
            e = [jnp.exp2((t - mx) * c_exp) for t in logits]
            inv = 1.0 / functools.reduce(jnp.add, e)
            probs[r] = [t * inv for t in e]
            return probs[r] if full_p else [inv]

        oa = {}

        def attn_mix(r, j):
            out = lambda r0, jj: functools.reduce(jnp.add, [probs[r0][w] * window(2, jj, r0, w) for w in range(W)])
            oa[r, j] = _a_ops(out(r, j), out(r, j + 4), out(TH + r, j), out(TH + r, j + 4))
            return oa[r, j]

        def get_xa(p, lo=0, hi=TH):
            return jnp.concatenate([xa[r][p] for r in range(lo, hi, 16)], axis=0)

        def get_oa(p):
            return jnp.concatenate([jnp.concatenate([oa[r % (16 * n_units), j][p] for j in range(4)], axis=1)
                                    for r in range(0, TH, 16)], axis=0)

        riders = []

        def paced(a, work):
            a = pltpu.bitcast(a, U32)
            step = a.shape[0] // 8 // len(work) * 8
            slabs = [a[:step // 16 * 8]] if step >= 16 else []
            for i, f in enumerate(work):
                lo = step // 16 * 8 + i * step
                slab = a[lo:lo + step if i + 1 < len(work) else a.shape[0]]
                head = jnp.concatenate([slab[0:8, 0:128] | _zero_after(f()), slab[0:8, 128:]], axis=1)
                slabs += [head, slab[8:]] if slab.shape[0] > 8 else [head]
            return pltpu.bitcast(jnp.concatenate(slabs, axis=0), BF)

        def mm(a, b):
            if not riders:
                return _dot(a, b)
            n = 128 * 512 // b.shape[0]
            outs = []
            for c in range(0, b.shape[1], n):
                work = riders.pop(0) if riders else ()
                outs.append(_dot(paced(a, work) if work else a, b[:, c:c + n]))
            return jnp.concatenate(outs, axis=1)

        def ride(work, n, skip=0):
            assert not riders
            if n == 0:
                for f in work:
                    f()
                return
            riders.extend([()] * skip)
            riders.extend(work[i * len(work) // n:(i + 1) * len(work) // n] for i in range(n))

        def up_ops(w_s, c):
            return _b_ops(*_quadrants(w_s, 0, KH, c_off[c], chunks[c] // 2))

        def up_proj(bops, lo=0, hi=TH):
            q = {}
            _strassen(lambda p: mm(get_xa(p, lo, hi), bops[p]()), q.__setitem__)
            return [q[i] for i in range(4)]

        def hidden(g, u):
            return _a_ops(*[_gelu_mul(a, b) for a, b in zip(g, u)])

        def down_ops(c):
            return _b_ops(*_quadrants(wd_s, c_off[c], chunks[c] // 2, 0, KH))

        def down(dops, ha, acc):
            out = {}
            for p in ORDER:
                v = mm(ha[p], dops[p]())
                out[p] = v if acc is None else acc[p] + v
            return out

        def project(t):
            def emit(i, quad):
                row0, j0 = (i // 2) * TH, (i % 2) * 4
                for j in range(4):
                    blk = quad[:, j * 128:(j + 1) * 128]
                    qkv_s[t, j0 + j, HALO + row0:HALO + row0 + TH, :] = blk
                    if row0 == 0 and t > 0:
                        qkv_s[t, j0 + j, 0:HALO, :] = jnp.broadcast_to(blk[0:1, :], (HALO, 128))
            w = jnp.concatenate([wp[t, r] for r in range(0, D, 16)], axis=0)
            bops = _b_ops(*(_quadrants(wqkv_s, 0, KH, t * D, KH) if inplace else _quadrants(w, 0, KH, 0, KH)))
            _strassen(lambda p: mm(get_xa(p), bops[p]()), emit)

        def ffn_copies(lo, hi, group):
            return [cols(wg_hbm, wg_s, lo, hi, group), cols(wu_hbm, wu_s, lo, hi, group),
                    rows(wd_hbm, wd_s, lo, hi, group)]

        def x_copies(lo, hi, group):
            return [rows(x_hbm, x_s, t + lo, t + hi, group) for t in (0, TH)]

        def pin(*vals):
            wof_s[7, 0:8, :] = pltpu.bitcast(_zero_after(vals), F32)

        def finish_early(vals, pending):
            wait(pending)
            x_s[0:TH, 0:KH] = functools.reduce(jnp.add, vals).astype(BF)
            cp = copy(x_s.at[0:TH, 0:128], out_hbm.at[0:TH, 0:128], 7)
            cp.start()
            cp.wait()

        b1, b2, b3, b4 = b_off[1:5]

        def first(hbm, vmem, group):
            if not halves:
                return [cols(hbm, vmem, 0, c_off[1], group)]
            return [copy(hbm.at[r:r + KH, 0:c_off[1]], vmem.at[r:r + KH, 0:c_off[1]], group) for r in (0, KH)]
        fh = c_off[1] // 2
        loads = [x_copies(0, b1, 0),
                 first(wg_hbm, wg_s, 1),
                 first(wu_hbm, wu_s, 2) + x_copies(b1, b2, 2),
                 x_copies(b2, b4, 3),
                 x_copies(b4, TH, 4) + [rows(wd_hbm, wd_s, 0, c_off[1], 4)],
                 ffn_copies(c_off[1], c_off[2], 5) + [copy(wqkv_hbm, wqkv_s, 5)],
                 [copy(wo_hbm, wo_s, 6)] + ffn_copies(c_off[2], DFU, 6)]
        if early & 1:
            loads[0] = [x_copies(0, x0a, 0), x_copies(x0a, b1, 8)]
        if early & 2:
            loads[1] = [[cols(wg_hbm, wg_s, fh, 2 * fh, 1)], [cols(wg_hbm, wg_s, 0, fh, 9)]]
        if stop == 'c0':
            loads[5:] = [], []
        grp1, grp2 = loads[5:]
        cat = lambda parts: [jnp.concatenate(t, axis=0) for t in zip(*parts)]
        ln_work = lambda lo, hi: [functools.partial(ln_unit, r) for r in range(lo, hi, 16)]

        def take(quads, lo, hi):
            return [t[lo:hi] for t in quads]

        def xa_vals(lo, hi):
            return [a for r in range(lo, hi, 16) for a in xa[r]]

        with scope("c0"):
            flat = lambda t: sum(map(flat, t), []) if isinstance(t, list) else [t]
            start(flat(loads))
            if early & 1:
                wait(loads[0][0])
                ride(ln_work(0, x0a), 0)
                pin(*xa_vals(0, x0a))
                wait(loads[0][1])
                ride(ln_work(x0a, b1), 0)
                pin(*xa_vals(x0a, b1))
            else:
                wait(loads[0])
                ride(ln_work(0, b1), 0)
                pin(*xa_vals(0, b1))
            gops, uops = _once(up_ops(wg_s, 0)), _once(up_ops(wu_s, 0))
            dops = _once(down_ops(0))
            block = lambda lo, hi: hidden(up_proj(gops, lo, hi), up_proj(uops, lo, hi))
            if early & 2:
                wait(loads[1][0])

                def prod(p):
                    if p == ORDER[2]:
                        wait(loads[1][1])
                    return mm(get_xa(p, 0, b1), gops[p]())
                q = {}
                _strassen(prod, q.__setitem__)
                g = [q[i] for i in range(4)]
            else:
                wait(loads[1])
                g = up_proj(gops, 0, b1)
            wait(loads[2])
            ride(ln_work(b1, b2), 0)
            hs = [hidden(g, up_proj(uops, 0, b1))]
            pin(*(xa_vals(b1, b2) + (hs[0] if pin_h & 1 else [])))
            wait(loads[3])
            ride(ln_work(b2, b4), 0)
            hs += [block(lo, hi) for lo, hi in zip((b1,) + mid, mid + (b3,))]
            pin(*(xa_vals(b3, b4) + (sum(hs[1:], []) if pin_h & 2 else [])))
            wait(loads[4])
            ride(ln_work(b4, TH), 0)
            tail = list(zip((b3,) + last, last + (TH,)))
            if split:
                hs2 = [block(*tail[0])]
                acc0 = down(dops, cat(hs), None)
                hs2 += [block(*t) for t in tail[1:]]
                acc1 = down(dops, cat(hs2), None)
                acc = {p: jnp.concatenate([acc0[p], acc1[p]], axis=0) for p in ORDER}
            else:
                acc = down(dops, cat(hs + [block(*t) for t in tail]), None)
        if stop == "c0":
            return finish_early(list(acc.values()), grp1 + grp2)

        with scope("c1"):
            wait(grp1)
            ride([functools.partial(permute_cols, t, r) for t in range(3) for r in range(0, D, 16)], perm_n, 2)
            acc = down(down_ops(1), hidden(up_proj(up_ops(wg_s, 1)), up_proj(up_ops(wu_s, 1))), acc)
            for t in range(3):
                project(t)
        if stop == "c1":
            return finish_early(list(acc.values()), grp2)

        with scope("ffn"):
            wait(grp2)
            done = []
            for r in range(0, 16 * n_units, 16):
                for t in (0, TH):
                    dep = _zero_after(done[-lag]) if lag and len(done) >= lag else None
                    done.append(attn_probs(t + r, dep))
            work = [functools.partial(permute_wo, j) for j in range(8)]
            work += [functools.partial(attn_mix, r, j) for r in range(0, 16 * n_units, 16) for j in range(4)]
            n_ride = (wo_at if wo_at is not None else len(chunks)) - pv_from
            for c in range(2, len(chunks)):
                n = c - pv_from
                if 0 <= n < n_ride:
                    ride(work[n * len(work) // n_ride:(n + 1) * len(work) // n_ride], pv_n)
                g = up_proj(up_ops(wg_s, c))
                if c == wo_at:
                    bops = _b_ops(*_quadrants(jnp.concatenate([wop[j] for j in range(8)], axis=1), 0, KH, 0, KH))
                    acc = {p: acc[p] + mm(get_oa(p), bops[p]()) for p in ORDER}
                ha = hidden(g, up_proj(up_ops(wu_s, c)))
                if c + 1 < len(chunks) or wo_at is None:
                    acc = down(down_ops(c), ha, acc)

            out_cps = []
            for j in range(KH // NO):
                lo, hi = slice(j * NO, (j + 1) * NO), slice(KH + j * NO, KH + (j + 1) * NO)
                if wo_at is None:
                    w_s, r0, k, lhs = jnp.concatenate([wop[i] for i in range(8)], axis=1), 0, KH, get_oa
                else:
                    w_s, r0, k, lhs = wd_s, c_off[-2], chunks[-1] // 2, lambda p: ha[p]
                bops = _b_ops(lambda: w_s[r0:r0 + k, lo], lambda: w_s[r0:r0 + k, hi],
                              lambda: w_s[r0 + k:r0 + 2 * k, lo], lambda: w_s[r0 + k:r0 + 2 * k, hi])

                def emit(i, quad):
                    rs, cs = slice((i // 2) * TH, (i // 2 + 1) * TH), (lo, hi)[i % 2]
                    x_s[rs, cs] = (x_s[rs, cs].astype(F32) + quad).astype(BF)
                    out_cps.append(copy(x_s.at[rs, cs], out_hbm.at[rs, cs], 7))
                    out_cps[-1].start()
                _strassen(lambda p: acc[p][:, lo] + mm(lhs(p), bops[p]()), emit)
            wait(out_cps)

    def fn(A_x, A_wqkv, A_wo, B_x, B_w_gate, B_w_up, B_w_down):
        del B_x
        hbm = pl.BlockSpec(memory_space=pl.ANY)
        out = pl.pallas_call(
            kernel,
            in_specs=[hbm] * 6,
            out_specs=hbm,
            out_shape=jax.ShapeDtypeStruct((S, D), BF),
            scratch_shapes=[
                pltpu.VMEM((S, D), BF),
                pltpu.VMEM((D, 3 * D), BF),
                pltpu.VMEM((3, 8, HALO + S, 128), F32),
                pltpu.VMEM((D, DF), BF),
                pltpu.VMEM((D, DF), BF),
                pltpu.VMEM((DF, D), BF),
                pltpu.VMEM((D, D), BF),
                pltpu.VMEM((8, H * STR, 128), F32),
                pltpu.SemaphoreType.DMA((10 if early else 8,)),
            ],
            compiler_params=pltpu.CompilerParams(vmem_limit_bytes=vmem_mb * 1024 * 1024, flags=flags),
        )(A_x.reshape(S, D), A_wqkv, A_wo, B_w_gate, B_w_up, B_w_down)
        return out.reshape(1, S, D)
    return fn


_impl = make(**dict(flags={'XLA_TPU_EVENLY_DISTRIBUTE_CRITICAL_NODES': True}))


@jax.jit
def pallas_parallel_sum__sliding_local_dilated__glu_gated_geglu__prompt_kernel(
    A_x: jax.Array,
    A_wqkv: jax.Array,
    A_wo: jax.Array,
    B_x: jax.Array,
    B_w_gate: jax.Array,
    B_w_up: jax.Array,
    B_w_down: jax.Array,
):
    return _impl(A_x, A_wqkv, A_wo, B_x, B_w_gate, B_w_up, B_w_down)
```

```python
import functools

import jax
import jax.experimental.pallas as pl
import jax.experimental.pallas.tpu as pltpu
import jax.numpy as jnp
import numpy as np

S, D, DF = 2048, 1024, 3584
H, DH, W, DIL = 32, 32, 8, 2
TH, KH = S // 2, D // 2
FC = 512
HALO = 16
STR = 33
LAG = 4
BF, F32, U32 = jnp.bfloat16, jnp.float32, jnp.uint32
ORDER = (4, 2, 1, 3, 0, 6, 5)


def _dot(a, b):
    return jnp.dot(a, b, preferred_element_type=F32)


def _left_ops(a11, a12, a21, a22):
    return [t.astype(BF) for t in (a11 + a22, a21 + a22, a11, a22, a11 + a12, a21 - a11, a12 - a22)]


def _right_ops(w, rows, cols):
    b11, b12, b21, b22 = (lambda r=r, c=c: w[r, c] for r in rows for c in cols)
    f = lambda t: t().astype(F32)
    return [lambda: (f(b11) + f(b22)).astype(BF), b11,
            lambda: (f(b12) - f(b22)).astype(BF),
            lambda: (f(b21) - f(b11)).astype(BF), b22,
            lambda: (f(b11) + f(b12)).astype(BF),
            lambda: (f(b21) + f(b22)).astype(BF)]


def _halves(start, size):
    return slice(start, start + size // 2), slice(start + size // 2, start + size)


def _strassen(product, emit):
    m5, m3 = product(4), product(2)
    emit(1, m3 + m5)
    m2, m4 = product(1), product(3)
    emit(2, m2 + m4)
    m1, m7 = product(0), product(6)
    emit(0, (m4 - m5) + m1 + m7)
    m6 = product(5)
    emit(3, (m3 - m2) + m1 + m6)


def _zero_after(values):
    tiles = []
    for v in values:
        v = pltpu.bitcast(v, U32)
        tiles += [v[r:r + 8, c:c + 128] for r in range(0, v.shape[0], 8) for c in range(0, v.shape[1], 128)]
    return (functools.reduce(jnp.bitwise_or, tiles) >> 31) >> 1


def _gelu_times(g, u):
    c = float(np.sqrt(2.0 / np.pi))
    z = g * (c + (c * 0.044715) * (g * g))
    return ((0.5 * g) * u) * (1.0 + jnp.tanh(z))


def _kernel(x_hbm, wqkv_hbm, wo_hbm, wg_hbm, wu_hbm, wd_hbm, out_hbm,
            x_s, wqkv_s, qkv_s, wg_s, wu_s, wd_s, wo_s, wot_s, sems):
    def copy(src, dst, index, group):
        return pltpu.make_async_copy(src.at[index], dst.at[index], sems.at[group])

    def x_rows(lo, hi, group):
        return [copy(x_hbm, x_s, (slice(t + lo, t + hi), slice(0, D)), group) for t in (0, TH)]

    def up_cols(hbm, vmem, lo, hi, group):
        return [copy(hbm, vmem, (slice(0, D), slice(lo, hi)), group)]

    def down_rows(lo, hi, group):
        return [copy(wd_hbm, wd_s, (slice(lo, hi), slice(0, D)), group)]

    def geglu_weights(lo, hi, group):
        return (up_cols(wg_hbm, wg_s, lo, hi, group) + up_cols(wu_hbm, wu_s, lo, hi, group)
                + down_rows(lo, hi, group))

    def wait(copies):
        for cp in copies:
            cp.wait()

    def pin(values):
        wot_s[7, 0:8, :] = pltpu.bitcast(_zero_after(values), F32)

    def layernorm(r):
        x = [x_s[r:r + 16, j * 128:(j + 1) * 128].astype(F32) for j in range(D // 128)]
        lane_sum = lambda t: jnp.broadcast_to(jnp.sum(t, axis=-1, keepdims=True), t.shape)
        mu = functools.reduce(jnp.add, x) * (128.0 / D)
        m2 = functools.reduce(jnp.add, [(t - mu) * (t - mu) for t in x])
        mean = lane_sum(mu) * (1.0 / 128)
        dm = mu - mean
        var = lane_sum(m2 + (D // 128) * (dm * dm)) * (1.0 / D)
        inv_std = jax.lax.rsqrt(var + 1e-5)
        return [(t - mean) * inv_std for t in x]

    xn_ops = {}

    def normalize(lo, hi):
        for r in range(lo, hi, 16):
            top, bot = layernorm(r), layernorm(TH + r)
            ops = [_left_ops(top[j], top[j + 4], bot[j], bot[j + 4]) for j in range(4)]
            xn_ops[r] = [jnp.concatenate(t, axis=1) for t in zip(*ops)]
        return [a for r in range(lo, hi, 16) for a in xn_ops[r]]

    def permute_columns(t, r):
        lane = jax.lax.broadcasted_iota(jnp.int32, (8, 128), 1)
        tiles = []
        for k in range(8):
            w = pltpu.bitcast(wqkv_s[r:r + 16, t * D + k * 128:t * D + (k + 1) * 128], U32)
            src = (lane - 4 * k) & 127
            idx = ((src & 3) << 5) | (src & 28) | (src >> 5)
            tiles.append(jnp.take_along_axis(w, idx, axis=1, mode="promise_in_bounds"))
        xs = [tiles[(-k) % 8] for k in range(8)]
        for b in range(3):
            sel = (lane & (4 << b)) != 0
            xs = [jnp.where(sel, xs[(k - (1 << b)) % 8], xs[k]) for k in range(8)]
        ys = [xs[j] if j == 0 else pltpu.roll(xs[j], 128 - 4 * j, 1) for j in range(8)]
        out = pltpu.bitcast(jnp.concatenate(ys, axis=1), BF)
        wqkv_s[r:r + 16, t * D:(t + 1) * D] = out
        return [out]

    def permuted_wo_tile(j):
        for h in range(H):
            wot_s[j, h * STR:h * STR + DH, :] = wo_s[h * DH:(h + 1) * DH, j * 128:(j + 1) * 128].astype(F32)
        return jnp.concatenate([wot_s[j, pl.ds(d, H, stride=STR), :].astype(BF) for d in range(DH)], axis=0)

    def window(t, j, r, w):
        return qkv_s[t, j, HALO + r - DIL * w:HALO + r - DIL * w + 16, :]

    def softmax_weights(r, after):
        scale = DH ** -0.5
        q = [window(0, j, r, 0) for j in range(8)]
        logits = []
        for w in range(W):
            pr = [q[j] * window(1, j, r, w) for j in range(8)]
            t = ((pr[0] + pr[1]) + (pr[2] + pr[3])) + ((pr[4] + pr[5]) + (pr[6] + pr[7]))
            if after is not None and w == 0:
                t = jnp.concatenate([pltpu.bitcast(pltpu.bitcast(t[0:8], U32) | after, F32), t[8:]], axis=0)
            t = t + pltpu.roll(t, 64, 1)
            t = t + pltpu.roll(t, 32, 1)
            if r < DIL * w:
                pos = r + jax.lax.broadcasted_iota(jnp.int32, (16, 128), 0)
                t = jnp.where(pos >= DIL * w, t, float(-1e9 / scale))
            logits.append(t)
        top = functools.reduce(jnp.maximum, logits)
        e = [jnp.exp2((t - top) * float(scale * np.log2(np.e))) for t in logits]
        inv = 1.0 / functools.reduce(jnp.add, e)
        return [t * inv for t in e]

    def attend(p, r, j):
        return functools.reduce(jnp.add, [p[w] * window(2, j, r, w) for w in range(W)])

    riders = []

    def paced(a, work):
        a = pltpu.bitcast(a, U32)
        step = a.shape[0] // 8 // len(work) * 8
        slabs = [a[:step // 16 * 8]] if step >= 16 else []
        for i, piece in enumerate(work):
            lo = step // 16 * 8 + i * step
            slab = a[lo:lo + step if i + 1 < len(work) else a.shape[0]]
            head = jnp.concatenate([slab[0:8, 0:128] | _zero_after(piece()), slab[0:8, 128:]], axis=1)
            slabs += [head, slab[8:]] if slab.shape[0] > 8 else [head]
        return pltpu.bitcast(jnp.concatenate(slabs, axis=0), BF)

    def matmul(a, b):
        if not riders:
            return _dot(a, b)
        n = 128 * 512 // b.shape[0]
        outs = []
        for c in range(0, b.shape[1], n):
            work = riders.pop(0) if riders else ()
            outs.append(_dot(paced(a, work) if work else a, b[:, c:c + n]))
        return jnp.concatenate(outs, axis=1)

    def xn_op(p, lo=0, hi=TH):
        return jnp.concatenate([xn_ops[r][p] for r in range(lo, hi, 16)], axis=0)

    def up_ops(w_s, c):
        return _right_ops(w_s, _halves(0, D), _halves(c * FC, FC))

    def down_ops(c):
        return _right_ops(wd_s, _halves(c * FC, FC), _halves(0, D))

    def up_proj(ops, lo=0, hi=TH, before=lambda p: None):
        quads = {}

        def product(p):
            before(p)
            return matmul(xn_op(p, lo, hi), ops[p]())
        _strassen(product, quads.__setitem__)
        return [quads[i] for i in range(4)]

    def hidden(g, u):
        return _left_ops(*[_gelu_times(a, b) for a, b in zip(g, u)])

    def down_proj(ops, h_ops, acc):
        out = {}
        for p in ORDER:
            v = matmul(h_ops[p], ops[p]())
            out[p] = v if acc is None else acc[p] + v
        return out

    def project(t, carry):
        def emit(i, quad):
            row0, j0 = (i // 2) * TH, (i % 2) * 4
            for j in range(4):
                blk = quad[:, j * 128:(j + 1) * 128]
                qkv_s[t, j0 + j, HALO + row0:HALO + row0 + TH, :] = blk
                if row0 == 0:
                    qkv_s[t, j0 + j, 0:HALO, :] = jnp.broadcast_to(blk[0:1, :], (HALO, 128))
        cols = (pl.ds(pl.multiple_of(t * D, D), KH), pl.ds(pl.multiple_of(t * D + KH, KH), KH))
        ops = _right_ops(wqkv_s, _halves(0, D), cols)
        _strassen(lambda p: matmul(xn_op(p), ops[p]()), emit)
        return carry

    edge = (0, 96, 192, 256, 448, 576, 704, TH)
    x0, x1 = x_rows(edge[0], edge[1], 0), x_rows(edge[1], edge[2], 1)
    gate_hi, gate_lo = up_cols(wg_hbm, wg_s, FC // 2, FC, 2), up_cols(wg_hbm, wg_s, 0, FC // 2, 3)
    second = up_cols(wu_hbm, wu_s, 0, FC, 4) + x_rows(edge[2], edge[3], 4)
    third = x_rows(edge[3], edge[5], 5)
    fourth = x_rows(edge[5], TH, 6) + down_rows(0, FC, 6)
    fifth = geglu_weights(FC, 2 * FC, 7) + [pltpu.make_async_copy(wqkv_hbm, wqkv_s, sems.at[7])]
    rest = [pltpu.make_async_copy(wo_hbm, wo_s, sems.at[8])] + geglu_weights(2 * FC, DF, 8)
    for cp in x0 + x1 + gate_hi + gate_lo + second + third + fourth + fifth + rest:
        cp.start()

    for j in range(8):
        wot_s[j, pl.ds(DH, H, stride=STR), :] = jnp.zeros((H, 128), F32)
        wot_s[j, H * STR:, :] = jnp.zeros((2 * DH, 128), F32)

    wait(x0)
    pin(normalize(edge[0], edge[1]))
    wait(x1)
    pin(normalize(edge[1], edge[2]))
    g_ops, u_ops, d_ops = ([functools.cache(f) for f in ops]
                           for ops in (up_ops(wg_s, 0), up_ops(wu_s, 0), down_ops(0)))
    block = lambda i: hidden(up_proj(g_ops, edge[i], edge[i + 1]), up_proj(u_ops, edge[i], edge[i + 1]))
    stack = lambda parts: [jnp.concatenate(t, axis=0) for t in zip(*parts)]
    wait(gate_hi)
    g = up_proj(g_ops, 0, edge[2], before=lambda p: wait(gate_lo) if p == ORDER[2] else None)
    wait(second)
    ahead = normalize(edge[2], edge[3])
    h = [hidden(g, up_proj(u_ops, 0, edge[2]))]
    pin(ahead)
    wait(third)
    ahead = normalize(edge[3], edge[5])
    h += [block(2), block(3)]
    pin(ahead[(edge[4] - edge[3]) // 16 * 7:])
    wait(fourth)
    normalize(edge[5], TH)
    h_late = [block(4)]
    acc0 = down_proj(d_ops, stack(h), None)
    h_late += [block(5), block(6)]
    acc1 = down_proj(d_ops, stack(h_late), None)
    acc = {p: jnp.concatenate([acc0[p], acc1[p]], axis=0) for p in ORDER}

    wait(fifth)
    work = [functools.partial(permute_columns, t, r) for t in range(3) for r in range(0, D, 16)]
    riders += [(), ()] + [work[i * len(work) // 40:(i + 1) * len(work) // 40] for i in range(40)]
    acc = down_proj(down_ops(1), hidden(up_proj(up_ops(wg_s, 1)), up_proj(up_ops(wu_s, 1))), acc)
    assert not riders
    jax.lax.fori_loop(0, 3, project, None)

    wait(rest)
    probs, done = {}, []
    for r in range(0, TH, 16):
        for t in (0, TH):
            probs[t + r] = softmax_weights(t + r, _zero_after(done[-LAG]) if len(done) >= LAG else None)
            done.append(probs[t + r])
    o_ops = {}
    for r in range(0, TH, 16):
        for j in range(4):
            o_ops[r, j] = _left_ops(attend(probs[r], r, j), attend(probs[r], r, j + 4),
                                    attend(probs[TH + r], TH + r, j), attend(probs[TH + r], TH + r, j + 4))
    for c in range(2, DF // FC):
        if c == 4:
            wo = jnp.concatenate([permuted_wo_tile(j) for j in range(8)], axis=1)
        acc = down_proj(down_ops(c), hidden(up_proj(up_ops(wg_s, c)), up_proj(up_ops(wu_s, c))), acc)

    def o_op(p):
        return jnp.concatenate([jnp.concatenate([o_ops[r, j][p] for j in range(4)], axis=1)
                                for r in range(0, TH, 16)], axis=0)

    stores = []
    for j in range(KH // 128):
        cols = (slice(j * 128, (j + 1) * 128), slice(KH + j * 128, KH + (j + 1) * 128))
        ops = _right_ops(wo, _halves(0, D), cols)

        def emit(i, quad):
            n = TH // 8 if (j, i) == (KH // 128 - 1, 3) else TH
            for r in range(0, TH, n):
                index = (slice((i // 2) * TH + r, (i // 2) * TH + r + n), cols[i % 2])
                x_s[index] = (x_s[index].astype(F32) + quad[r:r + n]).astype(BF)
                stores.append(copy(x_s, out_hbm, index, 9))
                stores[-1].start()
        _strassen(lambda p: acc[p][:, cols[0]] + matmul(o_op(p), ops[p]()), emit)
    wait(stores)


@jax.jit
def pallas_parallel_sum__sliding_local_dilated__glu_gated_geglu__prompt_kernel(
    A_x: jax.Array,
    A_wqkv: jax.Array,
    A_wo: jax.Array,
    B_x: jax.Array,
    B_w_gate: jax.Array,
    B_w_up: jax.Array,
    B_w_down: jax.Array,
):
    del B_x
    hbm = pl.BlockSpec(memory_space=pl.ANY)
    out = pl.pallas_call(
        _kernel,
        in_specs=[hbm] * 6,
        out_specs=hbm,
        out_shape=jax.ShapeDtypeStruct((S, D), BF),
        scratch_shapes=[
            pltpu.VMEM((S, D), BF),
            pltpu.VMEM((D, 3 * D), BF),
            pltpu.VMEM((3, 8, HALO + S, 128), F32),
            pltpu.VMEM((D, DF), BF),
            pltpu.VMEM((D, DF), BF),
            pltpu.VMEM((DF, D), BF),
            pltpu.VMEM((D, D), BF),
            pltpu.VMEM((8, H * STR + 2 * DH, 128), F32),
            pltpu.SemaphoreType.DMA((10,)),
        ],
        compiler_params=pltpu.CompilerParams(
            vmem_limit_bytes=127 * 1024 * 1024,
            flags={"XLA_TPU_EVENLY_DISTRIBUTE_CRITICAL_NODES": True},
        ),
    )(A_x.reshape(S, D), A_wqkv, A_wo, B_w_gate, B_w_up, B_w_down)
    return out.reshape(1, S, D)
```
